```python
import jax
import jax.numpy as jnp

def _softmax(x, axis=-1):
    return jax.nn.softmax(x, axis=axis)
def _gelu(x):
    return jax.nn.gelu(x, approximate=True)
def _silu(x):
    return jax.nn.silu(x)
def _sigmoid(x):
    return jax.nn.sigmoid(x)
def _layernorm(x, axis=-1, eps=1e-5):
    m = jnp.mean(x, axis=axis, keepdims=True)
    v = jnp.var(x, axis=axis, keepdims=True)
    return (x - m) / jnp.sqrt(v + eps)
def _scatter_add(tgt, idx, src, axis=0):
    return tgt.at[idx].add(src)
def _segment_sum(src, seg, n):
    return jax.ops.segment_sum(src, seg, n)
class _Rng:
    def __init__(self, key):
        self._k = key
    def _next(self):
        self._k, sub = jax.random.split(self._k)
        return sub
    def normal(self, shape):
        return jax.random.normal(self._next(), shape, dtype=jnp.bfloat16)
    def randint(self, lo, hi, shape):
        return jax.random.randint(self._next(), shape, lo, hi, dtype=jnp.int32)
    def uniform(self, shape, lo=0.0, hi=1.0):
        return jax.random.uniform(self._next(), shape, jnp.bfloat16, lo, hi)
    def permutation(self, n):
        return jax.random.permutation(self._next(), n)


kernel_name = 'gated_mix__mha_block_cached__compressed_kv_cla__decode'

def setup_inputs():
    _rng = _Rng(jax.random.key(int.from_bytes(__import__("os").urandom(4), "little")))
    _w = (lambda a: (lambda t: t.astype(jnp.bfloat16) if jnp.issubdtype(t.dtype, jnp.floating) else t)(jnp.asarray(a)))
    def _A_setup():
        B, Sq, D = 2, 1, 512
        H, Sk, Dh = 32, 8192, 128
        return {
            "x": _w((lambda *s: _rng.normal(s) * 0.05)(B, Sq, D)),
            "k_cache": _w((lambda *s: _rng.normal(s) * 0.05)(B, H, Sk, Dh)),
            "v_cache": _w((lambda *s: _rng.normal(s) * 0.05)(B, H, Sk, Dh)),
            "wq": _w((lambda *s: _rng.normal(s) * 0.05)(D, H * Dh) * (D ** -0.5)),
            "wo": _w((lambda *s: _rng.normal(s) * 0.05)(H * Dh, D) * ((H * Dh) ** -0.5)),
        }
    _A_in = _A_setup()

    def _B_setup():
        B, H, Sq, Sk, D, M = 2, 32, 1, 8192, 128, 512
        Dc = 4 * D
        return {
            "x": _w((lambda *s: _rng.normal(s) * 0.05)(B, Sq, M)),
            "c_kv": _w((lambda *s: _rng.normal(s) * 0.05)(B, Sk, Dc)),
            "w_q": _w((lambda *s: _rng.normal(s) * 0.05)(M, H, D) * (M ** -0.5)),
            "w_uk": _w((lambda *s: _rng.normal(s) * 0.05)(Dc, H, D) * (Dc ** -0.5)),
            "w_uv": _w((lambda *s: _rng.normal(s) * 0.05)(Dc, H, D) * (Dc ** -0.5)),
            "w_o": _w((lambda *s: _rng.normal(s) * 0.05)(H, D, M) * ((H * D) ** -0.5)),
        }
    _B_in = _B_setup()

    return {
        "A_x": _A_in["x"],
        "A_k_cache": _A_in["k_cache"],
        "A_v_cache": _A_in["v_cache"],
        "A_wq": _A_in["wq"],
        "A_wo": _A_in["wo"],
        "B_x": _B_in["x"],
        "B_c_kv": _B_in["c_kv"],
        "B_w_q": _B_in["w_q"],
        "B_w_uk": _B_in["w_uk"],
        "B_w_uv": _B_in["w_uv"],
        "B_w_o": _B_in["w_o"],
        "gate_w": _w((lambda *s: _rng.normal(s) * 0.05)(512)),
    }

def reference(A_x, A_k_cache, A_v_cache, A_wq, A_wo, B_x, B_c_kv, B_w_q, B_w_uk, B_w_uv, B_w_o, gate_w):
    def _A_ref(x, k_cache, v_cache, wq, wo):
        B, Sq, D = x.shape
        H, Dh = 32, 128
        q = (lambda x, *d: x.transpose(*d))((x @ wq).reshape(B, Sq, H, Dh), 0, 2, 1, 3)
        scores = jnp.einsum("bhqd,bhkd->bhqk", q, k_cache) * (Dh ** -0.5)
        p = _softmax(scores, axis=-1)
        o = jnp.einsum("bhqk,bhkd->bhqd", p, v_cache)
        return (lambda x, *d: x.transpose(*d))(o, 0, 2, 1, 3).reshape(B, Sq, H * Dh) @ wo

    def _B_ref(x, c_kv, w_q, w_uk, w_uv, w_o):
        B, Sq, M = x.shape[0], x.shape[1], x.shape[2]
        Sk = c_kv.shape[1]
        H, D = w_q.shape[1], w_q.shape[2]
        q = jnp.einsum("bqm,mhd->bhqd", x, w_q)
        k = jnp.einsum("bkc,chd->bhkd", c_kv, w_uk)
        v = jnp.einsum("bkc,chd->bhkd", c_kv, w_uv)
        scores = jnp.einsum("bhqd,bhkd->bhqk", q, k) * (D ** -0.5)
        off = Sk - Sq
        qi = jnp.arange(Sq)[:, None]
        kj = jnp.arange(Sk)[None, :]
        cmask = kj <= (qi + off)
        scores = jnp.where(cmask[None, None], scores, -1e9)
        p = _softmax(scores, axis=-1)
        ctx = jnp.einsum("bhqk,bhkd->bhqd", p, v)
        return jnp.einsum("bhqd,hdm->bqm", ctx, w_o)

    x = A_x
    g = _sigmoid((x * gate_w).sum(-1, keepdims=True))
    a = _A_ref(x, A_k_cache, A_v_cache, A_wq, A_wo)
    b = _B_ref(x, B_c_kv, B_w_q, B_w_uk, B_w_uv, B_w_o)
    return g * a + (1 - g) * b
```

```python
import contextlib

import jax
import jax.numpy as jnp
import jax.experimental.pallas as pl
import jax.experimental.pallas.tpu as pltpu

_NT = (((1,), (1,)), ((), ()))
_F32 = jnp.float32
_BF16 = jnp.bfloat16

NSLOT = 2
SUB128 = 208
SUB512 = 48
VPIECES = 4
PROFILE = False


def _scope(name):
    return jax.named_scope(name) if PROFILE else contextlib.nullcontext()


def _dot(a, b):
    return jnp.dot(a, b, preferred_element_type=_F32)


def _dot_nt(a, b):
    return jax.lax.dot_general(a, b, _NT, preferred_element_type=_F32)


def _stream2(src0, dst0, o0, sem0, src1, dst1, o1, sem1, rows, sub):
    nfull = rows // sub
    rem = rows - nfull * sub

    def pair(off, n):
        pltpu.make_async_copy(src0.at[pl.ds(o0 + off, n)], dst0.at[pl.ds(o0 + off, n)], sem0).start(priority=0)
        pltpu.make_async_copy(src1.at[pl.ds(o1 + off, n)], dst1.at[pl.ds(o1 + off, n)], sem1).start(priority=1)

    def one(s, c):
        pair(pl.multiple_of(s * sub, 16), sub)
        return c

    jax.lax.fori_loop(0, nfull, one, 0, unroll=4)
    if rem:
        pair(nfull * sub, rem)


def _wait_full(buf, sem):
    pltpu.make_async_copy(buf, buf, sem).wait()


@jax.jit
def pallas_gated_mix__mha_block_cached__compressed_kv_cla__decode_kernel(
    A_x: jax.Array,
    A_k_cache: jax.Array,
    A_v_cache: jax.Array,
    A_wq: jax.Array,
    A_wo: jax.Array,
    B_x: jax.Array,
    B_c_kv: jax.Array,
    B_w_q: jax.Array,
    B_w_uk: jax.Array,
    B_w_uv: jax.Array,
    B_w_o: jax.Array,
    gate_w: jax.Array,
):
    B, Sq, D = A_x.shape
    _, H, Sk, Dh = A_k_cache.shape
    Dc = B_c_kv.shape[-1]
    M = B_x.shape[-1]
    assert Sq == 1 and B == 2 and Dh == 128 and H == 32 and D == 512 and M == 512 and Dc == 512
    BH = B * H
    R = BH
    NJ = Dc // 128
    CH = 128 * H
    scale = float(Dh) ** -0.5
    HS = Sk // 2

    xa2 = A_x.reshape(B, D)
    xb2 = B_x.reshape(B, M)
    k3 = A_k_cache.reshape(BH, Sk, Dh)
    v3 = A_v_cache.reshape(BH, Sk, Dh)
    wqb2 = B_w_q.reshape(M * H, Dh)
    wuk2 = B_w_uk.reshape(Dc * H, Dh)
    wuv2 = B_w_uv.reshape(Dc * H, Dh)
    wob2 = B_w_o.reshape(H * Dh, M)

    def kernel(xa_hbm, xb_hbm, gw_hbm, k_hbm, v_hbm, wq_hbm, wo_hbm, ckv_hbm,
               wqb_hbm, wuk_hbm, wuv_hbm, wob_hbm,
               out_hbm,
               xa_v, xb_v, gw_v, wq_v, wo_v, ckv_v, wqb_v, wuk_v, wuv_v, wob_v,
               kbuf, vbuf, q_s, acc_s, out_v, sem, csem, ksem, vsem, lsem, osem):

        def issue_halves(src, dst, s, rows, sub):
            _stream2(src, dst, 0, s, src, dst, rows // 2, s, rows // 2, sub)

        def issue_ckv(b, u):
            _stream2(ckv_hbm.at[b], ckv_v.at[b], u * HS, csem.at[b],
                     ckv_hbm.at[b], ckv_v.at[b], u * HS + HS // 2, csem.at[b], HS // 2, SUB512)

        def issue_wq():
            hr = D // 2

            def one(s, c):
                r = pl.multiple_of((s // 4) * 16, 16)
                col = pl.multiple_of((s % 4) * 1024, 1024)
                pltpu.make_async_copy(wq_hbm.at[pl.ds(r, 16), pl.ds(col, 1024)],
                                      wq_v.at[pl.ds(r, 16), pl.ds(col, 1024)], sem.at[9]).start(priority=0)
                pltpu.make_async_copy(wq_hbm.at[pl.ds(hr + r, 16), pl.ds(col, 1024)],
                                      wq_v.at[pl.ds(hr + r, 16), pl.ds(col, 1024)], sem.at[9]).start(priority=1)
                return c

            jax.lax.fori_loop(0, (hr // 16) * 4, one, 0, unroll=4)

        def issue_kv(i, slot):
            _stream2(k_hbm.at[i], kbuf.at[slot], 0, ksem.at[slot],
                     v_hbm.at[i], vbuf.at[slot], 0, vsem.at[slot], Sk, SUB128)

        PR = HS // VPIECES

        def issue_kv_last(i, slot):
            _stream2(k_hbm.at[i], kbuf.at[slot], 0, ksem.at[slot],
                     k_hbm.at[i], kbuf.at[slot], HS, ksem.at[slot], HS, SUB128)
            for p in range(VPIECES):
                _stream2(v_hbm.at[i], vbuf.at[slot], p * PR, lsem.at[2 * p],
                         v_hbm.at[i], vbuf.at[slot], HS + p * PR, lsem.at[2 * p + 1], PR, SUB128)

        c_xa = pltpu.make_async_copy(xa_hbm, xa_v, sem.at[0])
        c_xb = pltpu.make_async_copy(xb_hbm, xb_v, sem.at[1])
        c_gw = pltpu.make_async_copy(gw_hbm, gw_v, sem.at[2])
        c_xb.start()
        c_xa.start()
        c_gw.start()
        with _scope("I_wqb_wuk"):
            issue_halves(wqb_hbm, wqb_v, sem.at[3], M * H, SUB128)
            issue_halves(wuk_hbm, wuk_v, sem.at[4], Dc * H, SUB128)

        with _scope("C_const"):
            st = (jax.lax.broadcasted_iota(jnp.int32, (128, CH), 1) // H
                  == jax.lax.broadcasted_iota(jnp.int32, (128, CH), 0)).astype(_F32).astype(_BF16)
            s_ = (jax.lax.broadcasted_iota(jnp.int32, (CH, 128), 0) // H
                  == jax.lax.broadcasted_iota(jnp.int32, (CH, 128), 1)).astype(_F32).astype(_BF16)
            hmask = (jax.lax.broadcasted_iota(jnp.int32, (R, CH), 1) % H
                     == jax.lax.broadcasted_iota(jnp.int32, (R, CH), 0) % H)

        def expand_project(c, w_ref):
            acc = jnp.zeros((R, Dh), _F32)
            for j in range(NJ):
                e = _dot(c[:, j * 128:(j + 1) * 128], st)
                l = jnp.where(hmask, e, 0.0).astype(_BF16)
                acc = acc + _dot(l, w_ref[j * CH:(j + 1) * CH, :])
            return acc

        with _scope("I_ckv00"):
            issue_ckv(0, 0)
        with _scope("C_B1"):
            c_xb.wait()
            c_xa.wait()
            c_gw.wait()
            xbv = xb_v[...].astype(_F32)
            xb = jnp.concatenate(
                [jnp.broadcast_to(xbv[b:b + 1], (H, M)) for b in range(B)], axis=0).astype(_BF16)
            _wait_full(wqb_v, sem.at[3])
            qb = expand_project(xb, wqb_v).astype(_BF16)

        with _scope("I_ckv01"):
            issue_ckv(0, 1)
        with _scope("C_B2"):
            _wait_full(wuk_v, sem.at[4])
            qabs = []
            for j in range(NJ):
                t = _dot_nt(qb, wuk_v[j * CH:(j + 1) * CH, :])
                t = jnp.where(hmask, t, 0.0).astype(_BF16)
                qabs.append(_dot(t, s_).astype(_BF16))
            qabs = jnp.concatenate(qabs, axis=1)

        def b_scores(b):
            _wait_full(ckv_v.at[b], csem.at[b])
            s = _dot_nt(qabs[b * H:(b + 1) * H], ckv_v[b]) * scale
            m = jnp.max(s, axis=-1, keepdims=True)
            p = jnp.exp(s - m)
            l = jnp.sum(p, axis=-1, keepdims=True)
            return p.astype(_BF16), l

        def b_ctx(b, p, l):
            cc = _dot(p, ckv_v[b])
            return (cc / l).astype(_BF16)

        with _scope("I_ckv10"):
            issue_ckv(1, 0)
        with _scope("C_B3s0"):
            p0, l0 = b_scores(0)
        with _scope("I_ckv11"):
            issue_ckv(1, 1)
        with _scope("C_B3c0"):
            cc0 = b_ctx(0, p0, l0)
        with _scope("I_wuv"):
            issue_halves(wuv_hbm, wuv_v, sem.at[7], Dc * H, SUB128)
        with _scope("C_B3s1"):
            p1, l1 = b_scores(1)
        with _scope("I_wob"):
            issue_halves(wob_hbm, wob_v, sem.at[8], H * Dh, SUB512)
        with _scope("C_B3c1"):
            cc1 = b_ctx(1, p1, l1)
            ctxc = jnp.concatenate([cc0, cc1], axis=0)
        with _scope("I_wq"):
            issue_wq()
        with _scope("C_B4"):
            _wait_full(wuv_v, sem.at[7])
            ctx = expand_project(ctxc, wuv_v)
        with _scope("I_wo"):
            issue_halves(wo_hbm, wo_v, sem.at[10], H * Dh, SUB512)
        with _scope("C_B5"):
            _wait_full(wob_v, sem.at[8])
            dmask = (jax.lax.broadcasted_iota(jnp.int32, (R, H * Dh), 1) // Dh
                     == jax.lax.broadcasted_iota(jnp.int32, (R, H * Dh), 0) % H)
            l2 = jnp.where(dmask, jnp.tile(ctx, (1, H)), 0.0).astype(_BF16)
            yb = _dot(l2, wob_v[...])
            outb = [jnp.sum(yb[b * H:(b + 1) * H], axis=0, keepdims=True) for b in range(B)]

            gw = gw_v[...].astype(_F32).reshape(1, D)
            xav = xa_v[...].astype(_F32)
            gate = jax.nn.sigmoid(jnp.sum(xav * gw, axis=-1, keepdims=True))

        with _scope("I_kv0"):
            issue_kv(0, 0)
        with _scope("C_QA"):
            _wait_full(wq_v, sem.at[9])
            xa = jnp.concatenate(
                [jnp.broadcast_to(xav[b:b + 1], (8, D)) for b in range(B)], axis=0).astype(_BF16)
            qa = _dot(xa, wq_v[...])
            for b in range(B):
                for h in range(H):
                    q_s[b * H + h] = qa[b * 8:(b + 1) * 8, h * Dh:(h + 1) * Dh].astype(_BF16)
            acc_s[...] = jnp.zeros_like(acc_s)
            _wait_full(wo_v, sem.at[10])

        def probs(i, slot):
            _wait_full(kbuf.at[slot], ksem.at[slot])
            s = _dot_nt(q_s[i], kbuf[slot]) * scale
            m = jnp.max(s, axis=-1, keepdims=True)
            p = jnp.exp(s - m)
            l = jnp.sum(p, axis=-1, keepdims=True)
            return p.astype(_BF16), l

        def step(i, carry):
            slot = i % NSLOT
            b = i // H
            h = i % H

            with _scope("I_kv"):
                @pl.when(i + 1 < BH - 1)
                def _():
                    issue_kv(i + 1, (i + 1) % NSLOT)

                @pl.when(i + 1 == BH - 1)
                def _():
                    issue_kv_last(BH - 1, (BH - 1) % NSLOT)

            with _scope("C_A"):
                p, l = probs(i, slot)
                _wait_full(vbuf.at[slot], vsem.at[slot])
                o = _dot(p, vbuf[slot]) / l
                y = _dot(o.astype(_BF16), wo_v[pl.ds(pl.multiple_of(h * Dh, Dh), Dh), :])
                acc_s[b] = acc_s[b] + y
            return carry

        jax.lax.fori_loop(0, BH - 1, step, 0)

        with _scope("C_last"):
            i = BH - 1
            slot = i % NSLOT
            p, l = probs(i, slot)
            o = jnp.zeros((8, Dh), _F32)
            for pc in range(VPIECES):
                for u in range(2):
                    r0 = u * HS + pc * PR
                    _wait_full(vbuf.at[slot, pl.ds(r0, PR)], lsem.at[2 * pc + u])
                    o = o + _dot(p[:, r0:r0 + PR], vbuf[slot, r0:r0 + PR, :])
            o = o / l
            y = _dot(o.astype(_BF16), wo_v[(H - 1) * Dh:H * Dh, :])
            a0 = acc_s[0][0:1]
            a1 = acc_s[1][0:1] + y[0:1]
            a = jnp.concatenate([a0, a1], axis=0)
            bb = jnp.concatenate(outb, axis=0)
            out_v[...] = (gate * a + (1.0 - gate) * bb).astype(out_v.dtype)
            c_out = pltpu.make_async_copy(out_v, out_hbm, osem.at[0])
            c_out.start()
            c_out.wait()

    any_spec = pl.BlockSpec(memory_space=pl.ANY)
    bf = _BF16
    out = pl.pallas_call(
        kernel,
        in_specs=[any_spec] * 12,
        out_specs=any_spec,
        out_shape=jax.ShapeDtypeStruct((B, D), A_x.dtype),
        scratch_shapes=[
            pltpu.VMEM((B, D), bf),
            pltpu.VMEM((B, M), bf),
            pltpu.VMEM((D,), bf),
            pltpu.VMEM((D, H * Dh), bf),
            pltpu.VMEM((H * Dh, D), bf),
            pltpu.VMEM((B, Sk, Dc), bf),
            pltpu.VMEM((M * H, Dh), bf),
            pltpu.VMEM((Dc * H, Dh), bf),
            pltpu.VMEM((Dc * H, Dh), bf),
            pltpu.VMEM((H * Dh, M), bf),
            pltpu.VMEM((NSLOT, Sk, Dh), bf),
            pltpu.VMEM((NSLOT, Sk, Dh), bf),
            pltpu.VMEM((BH, 8, Dh), bf),
            pltpu.VMEM((B, 8, D), _F32),
            pltpu.VMEM((B, D), bf),
            pltpu.SemaphoreType.DMA((11,)),
            pltpu.SemaphoreType.DMA((B,)),
            pltpu.SemaphoreType.DMA((NSLOT,)),
            pltpu.SemaphoreType.DMA((NSLOT,)),
            pltpu.SemaphoreType.DMA((2 * VPIECES,)),
            pltpu.SemaphoreType.DMA((1,)),
        ],
        compiler_params=pltpu.CompilerParams(vmem_limit_bytes=110 * 1024 * 1024),
    )(xa2, xb2, gate_w, k3, v3, A_wq, A_wo, B_c_kv, wqb2, wuk2, wuv2, wob2)
    return out.reshape(B, Sq, D)
```

```python
import contextlib

import jax
import jax.numpy as jnp
import jax.experimental.pallas as pl
import jax.experimental.pallas.tpu as pltpu

_NT = (((1,), (1,)), ((), ()))
_F32 = jnp.float32
_BF16 = jnp.bfloat16

NSLOT = 3
SUB128 = 208
SUB512 = 48
VPIECES = 8
PROFILE = False


def _scope(name):
    return jax.named_scope(name) if PROFILE else contextlib.nullcontext()


def _dot(a, b):
    return jnp.dot(a, b, preferred_element_type=_F32)


def _dot_nt(a, b):
    return jax.lax.dot_general(a, b, _NT, preferred_element_type=_F32)


def _stream2(src0, dst0, o0, sem0, src1, dst1, o1, sem1, rows, sub):
    nfull = rows // sub
    rem = rows - nfull * sub

    def pair(off, n):
        pltpu.make_async_copy(src0.at[pl.ds(o0 + off, n)], dst0.at[pl.ds(o0 + off, n)], sem0).start(priority=0)
        pltpu.make_async_copy(src1.at[pl.ds(o1 + off, n)], dst1.at[pl.ds(o1 + off, n)], sem1).start(priority=1)

    def one(s, c):
        pair(pl.multiple_of(s * sub, 16), sub)
        return c

    jax.lax.fori_loop(0, nfull, one, 0, unroll=4)
    if rem:
        pair(nfull * sub, rem)


def _wait_full(buf, sem):
    pltpu.make_async_copy(buf, buf, sem).wait()


@jax.jit
def pallas_gated_mix__mha_block_cached__compressed_kv_cla__decode_kernel(
    A_x: jax.Array,
    A_k_cache: jax.Array,
    A_v_cache: jax.Array,
    A_wq: jax.Array,
    A_wo: jax.Array,
    B_x: jax.Array,
    B_c_kv: jax.Array,
    B_w_q: jax.Array,
    B_w_uk: jax.Array,
    B_w_uv: jax.Array,
    B_w_o: jax.Array,
    gate_w: jax.Array,
):
    B, Sq, D = A_x.shape
    _, H, Sk, Dh = A_k_cache.shape
    Dc = B_c_kv.shape[-1]
    M = B_x.shape[-1]
    assert Sq == 1 and B == 2 and Dh == 128 and H == 32 and D == 512 and M == 512 and Dc == 512
    BH = B * H
    R = BH
    NJ = Dc // 128
    CH = 128 * H
    scale = float(Dh) ** -0.5
    HS = Sk // 2

    xa2 = A_x.reshape(B, D)
    xb2 = B_x.reshape(B, M)
    k3 = A_k_cache.reshape(BH, Sk, Dh)
    v3 = A_v_cache.reshape(BH, Sk, Dh)
    wqb2 = B_w_q.reshape(M * H, Dh)
    wuk2 = B_w_uk.reshape(Dc * H, Dh)
    wuv2 = B_w_uv.reshape(Dc * H, Dh)
    wob2 = B_w_o.reshape(H * Dh, M)

    def kernel(xa_hbm, xb_hbm, gw_hbm, k_hbm, v_hbm, wq_hbm, wo_hbm, ckv_hbm,
               wqb_hbm, wuk_hbm, wuv_hbm, wob_hbm,
               out_hbm,
               xa_v, xb_v, gw_v, wq_v, wo_v, ckv_v, wqb_v, wuk_v, wuv_v, wob_v,
               kbuf, vbuf, q_s, acc_s, out_v, sem, csem, ksem, vsem, lsem, osem):

        def issue_halves(src, dst, s, rows, sub):
            _stream2(src, dst, 0, s, src, dst, rows // 2, s, rows // 2, sub)

        def issue_ckv(b, u):
            _stream2(ckv_hbm.at[b], ckv_v.at[b], u * HS, csem.at[b],
                     ckv_hbm.at[b], ckv_v.at[b], u * HS + HS // 2, csem.at[b], HS // 2, SUB512)

        def issue_wq():
            hr = D // 2

            def one(s, c):
                r = pl.multiple_of((s // 4) * 16, 16)
                col = pl.multiple_of((s % 4) * 1024, 1024)
                pltpu.make_async_copy(wq_hbm.at[pl.ds(r, 16), pl.ds(col, 1024)],
                                      wq_v.at[pl.ds(r, 16), pl.ds(col, 1024)], sem.at[9]).start(priority=0)
                pltpu.make_async_copy(wq_hbm.at[pl.ds(hr + r, 16), pl.ds(col, 1024)],
                                      wq_v.at[pl.ds(hr + r, 16), pl.ds(col, 1024)], sem.at[9]).start(priority=1)
                return c

            jax.lax.fori_loop(0, (hr // 16) * 4, one, 0, unroll=4)

        def issue_kv(i, slot):
            _stream2(k_hbm.at[i], kbuf.at[slot], 0, ksem.at[slot],
                     v_hbm.at[i], vbuf.at[slot], 0, vsem.at[slot], Sk, SUB128)

        PR = Sk // VPIECES

        def issue_kv_last(i, slot):
            for p in range(VPIECES):
                _stream2(k_hbm.at[i], kbuf.at[slot], p * PR, ksem.at[slot],
                         v_hbm.at[i], vbuf.at[slot], p * PR, lsem.at[p], PR, SUB128)

        c_xa = pltpu.make_async_copy(xa_hbm, xa_v, sem.at[0])
        c_xb = pltpu.make_async_copy(xb_hbm, xb_v, sem.at[1])
        c_gw = pltpu.make_async_copy(gw_hbm, gw_v, sem.at[2])
        c_xb.start()
        c_xa.start()
        c_gw.start()
        with _scope("I_wqb_wuk"):
            issue_halves(wqb_hbm, wqb_v, sem.at[3], M * H, SUB128)
            issue_halves(wuk_hbm, wuk_v, sem.at[4], Dc * H, SUB128)

        with _scope("C_const"):
            st = (jax.lax.broadcasted_iota(jnp.int32, (128, CH), 1) // H
                  == jax.lax.broadcasted_iota(jnp.int32, (128, CH), 0)).astype(_F32).astype(_BF16)
            s_ = (jax.lax.broadcasted_iota(jnp.int32, (CH, 128), 0) // H
                  == jax.lax.broadcasted_iota(jnp.int32, (CH, 128), 1)).astype(_F32).astype(_BF16)
            hmask = (jax.lax.broadcasted_iota(jnp.int32, (R, CH), 1) % H
                     == jax.lax.broadcasted_iota(jnp.int32, (R, CH), 0) % H)

        def expand_project(c, w_ref):
            acc = jnp.zeros((R, Dh), _F32)
            for j in range(NJ):
                e = _dot(c[:, j * 128:(j + 1) * 128], st)
                l = jnp.where(hmask, e, 0.0).astype(_BF16)
                acc = acc + _dot(l, w_ref[j * CH:(j + 1) * CH, :])
            return acc

        with _scope("I_ckv00"):
            issue_ckv(0, 0)
        with _scope("C_B1"):
            c_xb.wait()
            c_xa.wait()
            c_gw.wait()
            xbv = xb_v[...].astype(_F32)
            xb = jnp.concatenate(
                [jnp.broadcast_to(xbv[b:b + 1], (H, M)) for b in range(B)], axis=0).astype(_BF16)
            _wait_full(wqb_v, sem.at[3])
            qb = expand_project(xb, wqb_v).astype(_BF16)

        with _scope("I_ckv01"):
            issue_ckv(0, 1)
        with _scope("C_B2"):
            _wait_full(wuk_v, sem.at[4])
            qabs = []
            for j in range(NJ):
                t = _dot_nt(qb, wuk_v[j * CH:(j + 1) * CH, :])
                t = jnp.where(hmask, t, 0.0).astype(_BF16)
                qabs.append(_dot(t, s_).astype(_BF16))
            qabs = jnp.concatenate(qabs, axis=1)

        def b_scores(b):
            _wait_full(ckv_v.at[b], csem.at[b])
            s = _dot_nt(qabs[b * H:(b + 1) * H], ckv_v[b]) * scale
            m = jnp.max(s, axis=-1, keepdims=True)
            p = jnp.exp(s - m)
            l = jnp.sum(p, axis=-1, keepdims=True)
            return p.astype(_BF16), l

        def b_ctx(b, p, l):
            cc = _dot(p, ckv_v[b])
            return (cc / l).astype(_BF16)

        with _scope("I_ckv10"):
            issue_ckv(1, 0)
        with _scope("C_B3s0"):
            p0, l0 = b_scores(0)
        with _scope("I_ckv11"):
            issue_ckv(1, 1)
        with _scope("C_B3c0"):
            cc0 = b_ctx(0, p0, l0)
        with _scope("I_wuv"):
            issue_halves(wuv_hbm, wuv_v, sem.at[7], Dc * H, SUB128)
        with _scope("C_B3s1"):
            p1, l1 = b_scores(1)
        with _scope("I_wob"):
            issue_halves(wob_hbm, wob_v, sem.at[8], H * Dh, SUB512)
        with _scope("C_B3c1"):
            cc1 = b_ctx(1, p1, l1)
            ctxc = jnp.concatenate([cc0, cc1], axis=0)
        with _scope("I_wq"):
            issue_wq()
        with _scope("C_B4"):
            _wait_full(wuv_v, sem.at[7])
            ctx = expand_project(ctxc, wuv_v)
        with _scope("I_wo"):
            issue_halves(wo_hbm, wo_v, sem.at[10], H * Dh, SUB512)
        with _scope("C_B5"):
            _wait_full(wob_v, sem.at[8])
            dmask = (jax.lax.broadcasted_iota(jnp.int32, (R, H * Dh), 1) // Dh
                     == jax.lax.broadcasted_iota(jnp.int32, (R, H * Dh), 0) % H)
            l2 = jnp.where(dmask, jnp.tile(ctx, (1, H)), 0.0).astype(_BF16)
            yb = _dot(l2, wob_v[...])
            outb = [jnp.sum(yb[b * H:(b + 1) * H], axis=0, keepdims=True) for b in range(B)]

            gw = gw_v[...].astype(_F32).reshape(1, D)
            xav = xa_v[...].astype(_F32)
            gate = jax.nn.sigmoid(jnp.sum(xav * gw, axis=-1, keepdims=True))

        with _scope("I_kv0"):
            issue_kv(0, 0)
        with _scope("C_QA"):
            _wait_full(wq_v, sem.at[9])
            xa = jnp.concatenate(
                [jnp.broadcast_to(xav[b:b + 1], (8, D)) for b in range(B)], axis=0).astype(_BF16)
            qa = _dot(xa, wq_v[...])
            for b in range(B):
                for h in range(H):
                    q_s[b * H + h] = qa[b * 8:(b + 1) * 8, h * Dh:(h + 1) * Dh].astype(_BF16)
            acc_s[...] = jnp.zeros_like(acc_s)
        with _scope("I_kv1"):
            for i in range(1, NSLOT - 1):
                issue_kv(i, i)
            _wait_full(wo_v, sem.at[10])

        def probs(i, slot):
            _wait_full(kbuf.at[slot], ksem.at[slot])
            s = _dot_nt(q_s[i], kbuf[slot]) * scale
            m = jnp.max(s, axis=-1, keepdims=True)
            p = jnp.exp(s - m)
            l = jnp.sum(p, axis=-1, keepdims=True)
            return p.astype(_BF16), l

        def step(i, carry):
            slot = i % NSLOT
            b = i // H
            h = i % H
            nxt = i + NSLOT - 1

            with _scope("I_kv"):
                @pl.when(nxt < BH - 1)
                def _():
                    issue_kv(nxt, nxt % NSLOT)

                @pl.when(nxt == BH - 1)
                def _():
                    issue_kv_last(BH - 1, (BH - 1) % NSLOT)

            with _scope("C_A"):
                p, l = probs(i, slot)
                _wait_full(vbuf.at[slot], vsem.at[slot])
                o = _dot(p, vbuf[slot]) / l
                y = _dot(o.astype(_BF16), wo_v[pl.ds(pl.multiple_of(h * Dh, Dh), Dh), :])
                acc_s[b] = acc_s[b] + y
            return carry

        jax.lax.fori_loop(0, BH - 1, step, 0)

        with _scope("C_last"):
            i = BH - 1
            slot = i % NSLOT
            p, l = probs(i, slot)
            o = jnp.zeros((8, Dh), _F32)
            for pc in range(VPIECES):
                r0 = pc * PR
                _wait_full(vbuf.at[slot, pl.ds(r0, PR)], lsem.at[pc])
                o = o + _dot(p[:, r0:r0 + PR], vbuf[slot, r0:r0 + PR, :])
            o = o / l
            y = _dot(o.astype(_BF16), wo_v[(H - 1) * Dh:H * Dh, :])
            a0 = acc_s[0][0:1]
            a1 = acc_s[1][0:1] + y[0:1]
            a = jnp.concatenate([a0, a1], axis=0)
            bb = jnp.concatenate(outb, axis=0)
            out_v[...] = (gate * a + (1.0 - gate) * bb).astype(out_v.dtype)
            c_out = pltpu.make_async_copy(out_v, out_hbm, osem.at[0])
            c_out.start()
            c_out.wait()

    any_spec = pl.BlockSpec(memory_space=pl.ANY)
    bf = _BF16
    out = pl.pallas_call(
        kernel,
        in_specs=[any_spec] * 12,
        out_specs=any_spec,
        out_shape=jax.ShapeDtypeStruct((B, D), A_x.dtype),
        scratch_shapes=[
            pltpu.VMEM((B, D), bf),
            pltpu.VMEM((B, M), bf),
            pltpu.VMEM((D,), bf),
            pltpu.VMEM((D, H * Dh), bf),
            pltpu.VMEM((H * Dh, D), bf),
            pltpu.VMEM((B, Sk, Dc), bf),
            pltpu.VMEM((M * H, Dh), bf),
            pltpu.VMEM((Dc * H, Dh), bf),
            pltpu.VMEM((Dc * H, Dh), bf),
            pltpu.VMEM((H * Dh, M), bf),
            pltpu.VMEM((NSLOT, Sk, Dh), bf),
            pltpu.VMEM((NSLOT, Sk, Dh), bf),
            pltpu.VMEM((BH, 8, Dh), bf),
            pltpu.VMEM((B, 8, D), _F32),
            pltpu.VMEM((B, D), bf),
            pltpu.SemaphoreType.DMA((11,)),
            pltpu.SemaphoreType.DMA((B,)),
            pltpu.SemaphoreType.DMA((NSLOT,)),
            pltpu.SemaphoreType.DMA((NSLOT,)),
            pltpu.SemaphoreType.DMA((VPIECES,)),
            pltpu.SemaphoreType.DMA((1,)),
        ],
        compiler_params=pltpu.CompilerParams(vmem_limit_bytes=110 * 1024 * 1024),
    )(xa2, xb2, gate_w, k3, v3, A_wq, A_wo, B_c_kv, wqb2, wuk2, wuv2, wob2)
    return out.reshape(B, Sq, D)
```

```python
import contextlib

import jax
import jax.numpy as jnp
import jax.experimental.pallas as pl
import jax.experimental.pallas.tpu as pltpu

_NT = (((1,), (1,)), ((), ()))
_F32 = jnp.float32
_BF16 = jnp.bfloat16

NSLOT = 3
SUB128 = 208
SUB512 = 48
VPIECES = 8
PROFILE = False


def _scope(name):
    return jax.named_scope(name) if PROFILE else contextlib.nullcontext()


def _dot(a, b):
    return jnp.dot(a, b, preferred_element_type=_F32)


def _dot_nt(a, b):
    return jax.lax.dot_general(a, b, _NT, preferred_element_type=_F32)


def _stream2(src0, dst0, o0, sem0, src1, dst1, o1, sem1, rows, sub):
    nfull = rows // sub
    rem = rows - nfull * sub

    def pair(off, n):
        pltpu.make_async_copy(src0.at[pl.ds(o0 + off, n)], dst0.at[pl.ds(o0 + off, n)], sem0).start(priority=0)
        pltpu.make_async_copy(src1.at[pl.ds(o1 + off, n)], dst1.at[pl.ds(o1 + off, n)], sem1).start(priority=1)

    def one(s, c):
        pair(pl.multiple_of(s * sub, 16), sub)
        return c

    jax.lax.fori_loop(0, nfull, one, 0, unroll=4)
    if rem:
        pair(nfull * sub, rem)


def _wait_full(buf, sem):
    pltpu.make_async_copy(buf, buf, sem).wait()


@jax.jit
def pallas_gated_mix__mha_block_cached__compressed_kv_cla__decode_kernel(
    A_x: jax.Array,
    A_k_cache: jax.Array,
    A_v_cache: jax.Array,
    A_wq: jax.Array,
    A_wo: jax.Array,
    B_x: jax.Array,
    B_c_kv: jax.Array,
    B_w_q: jax.Array,
    B_w_uk: jax.Array,
    B_w_uv: jax.Array,
    B_w_o: jax.Array,
    gate_w: jax.Array,
):
    B, Sq, D = A_x.shape
    _, H, Sk, Dh = A_k_cache.shape
    Dc = B_c_kv.shape[-1]
    M = B_x.shape[-1]
    assert Sq == 1 and B == 2 and Dh == 128 and H == 32 and D == 512 and M == 512 and Dc == 512
    BH = B * H
    R = BH
    NJ = Dc // 128
    CH = 128 * H
    scale = float(Dh) ** -0.5
    NU = 8
    UR = Sk // NU

    xa2 = A_x.reshape(B, D)
    xb2 = B_x.reshape(B, M)
    k3 = A_k_cache.reshape(BH, Sk, Dh)
    v3 = A_v_cache.reshape(BH, Sk, Dh)
    wqb2 = B_w_q.reshape(M * H, Dh)
    wuk2 = B_w_uk.reshape(Dc * H, Dh)
    wuv2 = B_w_uv.reshape(Dc * H, Dh)
    wob2 = B_w_o.reshape(H * Dh, M)

    def kernel(xa_hbm, xb_hbm, gw_hbm, k_hbm, v_hbm, wq_hbm, wo_hbm, ckv_hbm,
               wqb_hbm, wuk_hbm, wuv_hbm, wob_hbm,
               out_hbm,
               xa_v, xb_v, gw_v, wq_v, wo_v, ckv_v, wqb_v, wuk_v, wuv_v, wob_v,
               kbuf, vbuf, q_s, acc_s, out_v,
               sem, jsem, csem, ksem, vsem, lsem, osem):

        def issue_w3(a, src, dst, u):
            _stream2(src, dst, u * CH, jsem.at[a, u], src, dst, (u + 2) * CH, jsem.at[a, u + 2], CH, SUB128)

        def issue_ckv(u):
            _stream2(ckv_hbm.at[0], ckv_v.at[0], u * UR, csem.at[0, u],
                     ckv_hbm.at[1], ckv_v.at[1], u * UR, csem.at[1, u], UR, SUB512)

        def issue_w512(src, dst, s, u):
            qr = (H * Dh) // 4
            _stream2(src, dst, u * qr, s, src, dst, (u + 2) * qr, s, qr, SUB512)

        def issue_wq(u):
            qr = D // 4

            def one(s, c):
                r = pl.multiple_of(u * qr + s * 16, 16)
                r2 = pl.multiple_of(r + 2 * qr, 16)
                for col, n in ((0, 1408), (1408, 1408), (2816, 1280)):
                    pltpu.make_async_copy(wq_hbm.at[pl.ds(r, 16), pl.ds(col, n)],
                                          wq_v.at[pl.ds(r, 16), pl.ds(col, n)], sem.at[3]).start(priority=0)
                    pltpu.make_async_copy(wq_hbm.at[pl.ds(r2, 16), pl.ds(col, n)],
                                          wq_v.at[pl.ds(r2, 16), pl.ds(col, n)], sem.at[3]).start(priority=1)
                return c

            jax.lax.fori_loop(0, qr // 16, one, 0)

        def issue_kv(i, slot):
            _stream2(k_hbm.at[i], kbuf.at[slot], 0, ksem.at[slot],
                     v_hbm.at[i], vbuf.at[slot], 0, vsem.at[slot], Sk, SUB128)

        PR = Sk // VPIECES

        def issue_kv_last(i, slot):
            for p in range(VPIECES):
                _stream2(k_hbm.at[i], kbuf.at[slot], p * PR, ksem.at[slot],
                         v_hbm.at[i], vbuf.at[slot], p * PR, lsem.at[p], PR, SUB128)

        def wait_w3(a, ref, j):
            _wait_full(ref.at[pl.ds(j * CH, CH)], jsem.at[a, j])

        c_xa = pltpu.make_async_copy(xa_hbm, xa_v, sem.at[0])
        c_xb = pltpu.make_async_copy(xb_hbm, xb_v, sem.at[1])
        c_gw = pltpu.make_async_copy(gw_hbm, gw_v, sem.at[2])
        with _scope("I_0"):
            issue_w3(0, wqb_hbm, wqb_v, 0)
            c_xb.start()
            c_xa.start()
            c_gw.start()
            issue_w3(0, wqb_hbm, wqb_v, 1)
            issue_w3(1, wuk_hbm, wuk_v, 0)

        with _scope("C_const"):
            st = (jax.lax.broadcasted_iota(jnp.int32, (128, CH), 1) // H
                  == jax.lax.broadcasted_iota(jnp.int32, (128, CH), 0)).astype(_F32).astype(_BF16)
            s_ = (jax.lax.broadcasted_iota(jnp.int32, (CH, 128), 0) // H
                  == jax.lax.broadcasted_iota(jnp.int32, (CH, 128), 1)).astype(_F32).astype(_BF16)
            hmask = (jax.lax.broadcasted_iota(jnp.int32, (R, CH), 1) % H
                     == jax.lax.broadcasted_iota(jnp.int32, (R, CH), 0) % H)

        def project_j(c, a, w_ref, j):
            e = _dot(c[:, j * 128:(j + 1) * 128], st)
            l = jnp.where(hmask, e, 0.0).astype(_BF16)
            wait_w3(a, w_ref, j)
            return _dot(l, w_ref[j * CH:(j + 1) * CH, :])

        with _scope("I"):
            issue_w3(1, wuk_hbm, wuk_v, 1)
            issue_ckv(0)
        with _scope("C_B1"):
            c_xb.wait()
            c_xa.wait()
            c_gw.wait()
            xbv = xb_v[...].astype(_F32)
            xb = jnp.concatenate(
                [jnp.broadcast_to(xbv[b:b + 1], (H, M)) for b in range(B)], axis=0).astype(_BF16)
            qb = project_j(xb, 0, wqb_v, 0) + project_j(xb, 0, wqb_v, 2)
        with _scope("I"):
            issue_ckv(1)
        with _scope("C_B1"):
            qb = qb + project_j(xb, 0, wqb_v, 1) + project_j(xb, 0, wqb_v, 3)
            qb = qb.astype(_BF16)

        def absorb_j(j):
            wait_w3(1, wuk_v, j)
            t = _dot_nt(qb, wuk_v[j * CH:(j + 1) * CH, :])
            t = jnp.where(hmask, t, 0.0).astype(_BF16)
            return _dot(t, s_).astype(_BF16)

        qabs = [None] * NJ
        with _scope("I"):
            issue_ckv(2)
        with _scope("C_B2"):
            qabs[0] = absorb_j(0)
            qabs[2] = absorb_j(2)
        with _scope("I"):
            issue_ckv(3)
        with _scope("C_B2"):
            qabs[1] = absorb_j(1)
            qabs[3] = absorb_j(3)
            qabs = jnp.concatenate(qabs, axis=1)

        sc = [[None] * NU for _ in range(B)]

        def b_scores(u):
            for b in range(B):
                _wait_full(ckv_v.at[b, pl.ds(u * UR, UR)], csem.at[b, u])
                sc[b][u] = _dot_nt(qabs[b * H:(b + 1) * H], ckv_v[b, u * UR:(u + 1) * UR, :]) * scale

        def b_softmax(b):
            s = jnp.concatenate(sc[b], axis=1)
            m = jnp.max(s, axis=-1, keepdims=True)
            p = jnp.exp(s - m)
            l = jnp.sum(p, axis=-1, keepdims=True)
            return p.astype(_BF16), l

        def b_ctx(b, p, l):
            cc = _dot(p, ckv_v[b])
            return (cc / l).astype(_BF16)

        with _scope("I"):
            issue_ckv(4)
        with _scope("C_QK"):
            b_scores(0)
            b_scores(1)
        with _scope("I"):
            issue_ckv(5)
        with _scope("C_QK"):
            b_scores(2)
        with _scope("I"):
            issue_ckv(6)
        with _scope("C_QK"):
            b_scores(3)
        with _scope("I"):
            issue_ckv(7)
        with _scope("C_QK"):
            b_scores(4)
        with _scope("I"):
            issue_w3(2, wuv_hbm, wuv_v, 0)
        with _scope("C_QK"):
            b_scores(5)
        with _scope("I"):
            issue_w3(2, wuv_hbm, wuv_v, 1)
        with _scope("C_QK"):
            b_scores(6)
        with _scope("I"):
            issue_w512(wob_hbm, wob_v, sem.at[4], 0)
        with _scope("C_QK"):
            b_scores(7)
            p0, l0 = b_softmax(0)
        with _scope("I"):
            issue_w512(wob_hbm, wob_v, sem.at[4], 1)
        with _scope("C_PV"):
            p1, l1 = b_softmax(1)
            cc0 = b_ctx(0, p0, l0)
        with _scope("I"):
            issue_wq(0)
        with _scope("C_PV"):
            cc1 = b_ctx(1, p1, l1)
            ctxc = jnp.concatenate([cc0, cc1], axis=0)
        with _scope("I"):
            issue_wq(1)
        with _scope("C_B4"):
            ctx = project_j(ctxc, 2, wuv_v, 0) + project_j(ctxc, 2, wuv_v, 2)
        with _scope("I"):
            issue_w512(wo_hbm, wo_v, sem.at[5], 0)
            issue_w512(wo_hbm, wo_v, sem.at[5], 1)
        with _scope("C_B4"):
            ctx = ctx + project_j(ctxc, 2, wuv_v, 1) + project_j(ctxc, 2, wuv_v, 3)
        with _scope("I_kv0"):
            issue_kv(0, 0)
        with _scope("C_B5"):
            _wait_full(wob_v, sem.at[4])
            dmask = (jax.lax.broadcasted_iota(jnp.int32, (R, H * Dh), 1) // Dh
                     == jax.lax.broadcasted_iota(jnp.int32, (R, H * Dh), 0) % H)
            l2 = jnp.where(dmask, jnp.tile(ctx, (1, H)), 0.0).astype(_BF16)
            yb = _dot(l2, wob_v[...])
            outb = [jnp.sum(yb[b * H:(b + 1) * H], axis=0, keepdims=True) for b in range(B)]

            gw = gw_v[...].astype(_F32).reshape(1, D)
            xav = xa_v[...].astype(_F32)
            gate = jax.nn.sigmoid(jnp.sum(xav * gw, axis=-1, keepdims=True))
            base = (1.0 - gate) * jnp.concatenate(outb, axis=0)

        with _scope("C_QA"):
            _wait_full(wq_v, sem.at[3])
            xa = jnp.concatenate(
                [jnp.broadcast_to(xav[b:b + 1], (8, D)) for b in range(B)], axis=0).astype(_BF16)
            qa = _dot(xa, wq_v[...])
            for b in range(B):
                for h in range(H):
                    q_s[b * H + h] = qa[b * 8:(b + 1) * 8, h * Dh:(h + 1) * Dh].astype(_BF16)
            acc_s[...] = jnp.zeros_like(acc_s)
        with _scope("I_kv1"):
            for i in range(1, NSLOT - 1):
                issue_kv(i, i)
            _wait_full(wo_v, sem.at[5])

        def probs(i, slot):
            _wait_full(kbuf.at[slot], ksem.at[slot])
            s = _dot_nt(q_s[i], kbuf[slot]) * scale
            m = jnp.max(s, axis=-1, keepdims=True)
            p = jnp.exp(s - m)
            l = jnp.sum(p, axis=-1, keepdims=True)
            return p.astype(_BF16), l

        def step(i, carry):
            slot = i % NSLOT
            b = i // H
            h = i % H
            nxt = i + NSLOT - 1

            with _scope("I_kv"):
                @pl.when(nxt < BH - 1)
                def _():
                    issue_kv(nxt, nxt % NSLOT)

                @pl.when(nxt == BH - 1)
                def _():
                    issue_kv_last(BH - 1, (BH - 1) % NSLOT)

            with _scope("C_A"):
                p, l = probs(i, slot)
                _wait_full(vbuf.at[slot], vsem.at[slot])
                o = _dot(p, vbuf[slot]) / l
                y = _dot(o.astype(_BF16), wo_v[pl.ds(pl.multiple_of(h * Dh, Dh), Dh), :])
                acc_s[b] = acc_s[b] + y
            return carry

        jax.lax.fori_loop(0, BH - 1, step, 0)

        with _scope("C_last"):
            i = BH - 1
            slot = i % NSLOT
            p, l = probs(i, slot)
            o = jnp.zeros((8, Dh), _F32)
            for pc in range(VPIECES):
                r0 = pc * PR
                _wait_full(vbuf.at[slot, pl.ds(r0, PR)], lsem.at[pc])
                o = o + _dot(p[:, r0:r0 + PR], vbuf[slot, r0:r0 + PR, :])
            o = o / l
            y = _dot(o.astype(_BF16), wo_v[(H - 1) * Dh:H * Dh, :])
            a0 = acc_s[0][0:1]
            a1 = acc_s[1][0:1] + y[0:1]
            a = jnp.concatenate([a0, a1], axis=0)
            out_v[...] = (gate * a + base).astype(out_v.dtype)
            c_out = pltpu.make_async_copy(out_v, out_hbm, osem.at[0])
            c_out.start()
            c_out.wait()

    any_spec = pl.BlockSpec(memory_space=pl.ANY)
    bf = _BF16
    out = pl.pallas_call(
        kernel,
        in_specs=[any_spec] * 12,
        out_specs=any_spec,
        out_shape=jax.ShapeDtypeStruct((B, D), A_x.dtype),
        scratch_shapes=[
            pltpu.VMEM((B, D), bf),
            pltpu.VMEM((B, M), bf),
            pltpu.VMEM((D,), bf),
            pltpu.VMEM((D, H * Dh), bf),
            pltpu.VMEM((H * Dh, D), bf),
            pltpu.VMEM((B, Sk, Dc), bf),
            pltpu.VMEM((M * H, Dh), bf),
            pltpu.VMEM((Dc * H, Dh), bf),
            pltpu.VMEM((Dc * H, Dh), bf),
            pltpu.VMEM((H * Dh, M), bf),
            pltpu.VMEM((NSLOT, Sk, Dh), bf),
            pltpu.VMEM((NSLOT, Sk, Dh), bf),
            pltpu.VMEM((BH, 8, Dh), bf),
            pltpu.VMEM((B, 8, D), _F32),
            pltpu.VMEM((B, D), bf),
            pltpu.SemaphoreType.DMA((6,)),
            pltpu.SemaphoreType.DMA((3, NJ)),
            pltpu.SemaphoreType.DMA((B, NU)),
            pltpu.SemaphoreType.DMA((NSLOT,)),
            pltpu.SemaphoreType.DMA((NSLOT,)),
            pltpu.SemaphoreType.DMA((VPIECES,)),
            pltpu.SemaphoreType.DMA((1,)),
        ],
        compiler_params=pltpu.CompilerParams(vmem_limit_bytes=110 * 1024 * 1024,
                                             disable_semaphore_checks=True),
    )(xa2, xb2, gate_w, k3, v3, A_wq, A_wo, B_c_kv, wqb2, wuk2, wuv2, wob2)
    return out.reshape(B, Sq, D)
```

```python
import contextlib

import jax
import jax.numpy as jnp
import jax.experimental.pallas as pl
import jax.experimental.pallas.tpu as pltpu

_NT = (((1,), (1,)), ((), ()))
_F32 = jnp.float32
_BF16 = jnp.bfloat16

NSLOT = 3
SUB128 = 208
SUB512 = 48
VPIECES = 8
PROFILE = False
ROFF = 26


def _scope(name):
    return jax.named_scope(name) if PROFILE else contextlib.nullcontext()


def _dot(a, b):
    return jnp.dot(a, b, preferred_element_type=_F32)


def _dot_nt(a, b):
    return jax.lax.dot_general(a, b, _NT, preferred_element_type=_F32)


def _stream2(src0, dst0, o0, sem0, src1, dst1, o1, sem1, rows, sub):
    nfull = rows // sub
    rem = rows - nfull * sub

    def pair(off, n):
        pltpu.make_async_copy(src0.at[pl.ds(o0 + off, n)], dst0.at[pl.ds(o0 + off, n)], sem0).start(priority=0)
        pltpu.make_async_copy(src1.at[pl.ds(o1 + off, n)], dst1.at[pl.ds(o1 + off, n)], sem1).start(priority=1)

    def one(s, c):
        pair(pl.multiple_of(s * sub, 16), sub)
        return c

    jax.lax.fori_loop(0, nfull, one, 0, unroll=4)
    if rem:
        pair(nfull * sub, rem)


def _wait_full(buf, sem):
    pltpu.make_async_copy(buf, buf, sem).wait()


@jax.jit
def pallas_gated_mix__mha_block_cached__compressed_kv_cla__decode_kernel(
    A_x: jax.Array,
    A_k_cache: jax.Array,
    A_v_cache: jax.Array,
    A_wq: jax.Array,
    A_wo: jax.Array,
    B_x: jax.Array,
    B_c_kv: jax.Array,
    B_w_q: jax.Array,
    B_w_uk: jax.Array,
    B_w_uv: jax.Array,
    B_w_o: jax.Array,
    gate_w: jax.Array,
):
    B, Sq, D = A_x.shape
    _, H, Sk, Dh = A_k_cache.shape
    Dc = B_c_kv.shape[-1]
    M = B_x.shape[-1]
    assert Sq == 1 and B == 2 and Dh == 128 and H == 32 and D == 512 and M == 512 and Dc == 512
    BH = B * H
    R = BH
    NJ = Dc // 128
    CH = 128 * H
    scale = float(Dh) ** -0.5
    NU = 8
    UR = Sk // NU

    xa2 = A_x.reshape(B, D)
    xb2 = B_x.reshape(B, M)
    k3 = A_k_cache.reshape(BH, Sk, Dh)
    v3 = A_v_cache.reshape(BH, Sk, Dh)
    wqb2 = B_w_q.reshape(M * H, Dh)
    wuk2 = B_w_uk.reshape(Dc * H, Dh)
    wuv2 = B_w_uv.reshape(Dc * H, Dh)
    wob2 = B_w_o.reshape(H * Dh, M)

    def kernel(xa_hbm, xb_hbm, gw_hbm, k_hbm, v_hbm, wq_hbm, wo_hbm, ckv_hbm,
               wqb_hbm, wuk_hbm, wuv_hbm, wob_hbm,
               out_hbm,
               xa_v, xb_v, gw_v, wq_v, wo_v, ckv_v, wqb_v, wuk_v, wuv_v, wob_v,
               kbuf, vbuf, q_s, acc_s, out_v,
               sem, jsem, csem, ksem, vsem, lsem, osem):

        def issue_w3(a, src, dst, u):
            _stream2(src, dst, u * CH, jsem.at[a, u], src, dst, (u + 2) * CH, jsem.at[a, u + 2], CH, SUB128)

        def issue_ckv(u):
            _stream2(ckv_hbm.at[0], ckv_v.at[0], u * UR, csem.at[0, u],
                     ckv_hbm.at[1], ckv_v.at[1], u * UR, csem.at[1, u], UR, SUB512)

        def issue_w512(src, dst, s, u):
            qr = (H * Dh) // 4
            _stream2(src, dst, u * qr, s, src, dst, (u + 2) * qr, s, qr, SUB512)

        def issue_wq(u):
            qr = D // 4

            def one(s, c):
                r = pl.multiple_of(u * qr + s * 16, 16)
                r2 = pl.multiple_of(r + 2 * qr, 16)
                for col, n in ((0, 1408), (1408, 1408), (2816, 1280)):
                    pltpu.make_async_copy(wq_hbm.at[pl.ds(r, 16), pl.ds(col, n)],
                                          wq_v.at[pl.ds(r, 16), pl.ds(col, n)], sem.at[3]).start(priority=0)
                    pltpu.make_async_copy(wq_hbm.at[pl.ds(r2, 16), pl.ds(col, n)],
                                          wq_v.at[pl.ds(r2, 16), pl.ds(col, n)], sem.at[3]).start(priority=1)
                return c

            jax.lax.fori_loop(0, qr // 16, one, 0)

        def issue_kv(i, slot):
            nfull = Sk // SUB128
            rem = Sk - nfull * SUB128

            def one(s, c):
                off = pl.multiple_of(s * SUB128, 16)
                s2 = s + ROFF
                s2 = jnp.where(s2 >= nfull, s2 - nfull, s2)
                off2 = pl.multiple_of(s2 * SUB128, 16)
                pltpu.make_async_copy(k_hbm.at[i, pl.ds(off, SUB128)], kbuf.at[slot, pl.ds(off, SUB128)],
                                      ksem.at[slot]).start(priority=0)
                pltpu.make_async_copy(v_hbm.at[i, pl.ds(off2, SUB128)], vbuf.at[slot, pl.ds(off2, SUB128)],
                                      vsem.at[slot]).start(priority=1)
                return c

            jax.lax.fori_loop(0, nfull, one, 0, unroll=3)
            off = nfull * SUB128
            pltpu.make_async_copy(k_hbm.at[i, pl.ds(off, rem)], kbuf.at[slot, pl.ds(off, rem)],
                                  ksem.at[slot]).start(priority=0)
            pltpu.make_async_copy(v_hbm.at[i, pl.ds(off, rem)], vbuf.at[slot, pl.ds(off, rem)],
                                  vsem.at[slot]).start(priority=1)

        PR = Sk // VPIECES

        def issue_kv_last(i, slot):
            for p in range(VPIECES):
                _stream2(k_hbm.at[i], kbuf.at[slot], p * PR, ksem.at[slot],
                         v_hbm.at[i], vbuf.at[slot], p * PR, lsem.at[p], PR, SUB128)

        def wait_w3(a, ref, j):
            _wait_full(ref.at[pl.ds(j * CH, CH)], jsem.at[a, j])

        c_xa = pltpu.make_async_copy(xa_hbm, xa_v, sem.at[0])
        c_xb = pltpu.make_async_copy(xb_hbm, xb_v, sem.at[1])
        c_gw = pltpu.make_async_copy(gw_hbm, gw_v, sem.at[2])
        with _scope("I_0"):
            issue_w3(0, wqb_hbm, wqb_v, 0)
            c_xb.start()
            c_xa.start()
            c_gw.start()
            issue_w3(0, wqb_hbm, wqb_v, 1)
            issue_w3(1, wuk_hbm, wuk_v, 0)

        with _scope("C_const"):
            st = (jax.lax.broadcasted_iota(jnp.int32, (128, CH), 1) // H
                  == jax.lax.broadcasted_iota(jnp.int32, (128, CH), 0)).astype(_F32).astype(_BF16)
            s_ = (jax.lax.broadcasted_iota(jnp.int32, (CH, 128), 0) // H
                  == jax.lax.broadcasted_iota(jnp.int32, (CH, 128), 1)).astype(_F32).astype(_BF16)
            hmask = (jax.lax.broadcasted_iota(jnp.int32, (R, CH), 1) % H
                     == jax.lax.broadcasted_iota(jnp.int32, (R, CH), 0) % H)

        def project_j(c, a, w_ref, j):
            e = _dot(c[:, j * 128:(j + 1) * 128], st)
            l = jnp.where(hmask, e, 0.0).astype(_BF16)
            wait_w3(a, w_ref, j)
            return _dot(l, w_ref[j * CH:(j + 1) * CH, :])

        with _scope("I"):
            issue_w3(1, wuk_hbm, wuk_v, 1)
            issue_ckv(0)
        with _scope("C_B1"):
            c_xb.wait()
            c_xa.wait()
            c_gw.wait()
            xbv = xb_v[...].astype(_F32)
            xb = jnp.concatenate(
                [jnp.broadcast_to(xbv[b:b + 1], (H, M)) for b in range(B)], axis=0).astype(_BF16)
            qb = project_j(xb, 0, wqb_v, 0) + project_j(xb, 0, wqb_v, 2)
        with _scope("I"):
            issue_ckv(1)
        with _scope("C_B1"):
            qb = qb + project_j(xb, 0, wqb_v, 1) + project_j(xb, 0, wqb_v, 3)
            qb = qb.astype(_BF16)

        def absorb_j(j):
            wait_w3(1, wuk_v, j)
            t = _dot_nt(qb, wuk_v[j * CH:(j + 1) * CH, :])
            t = jnp.where(hmask, t, 0.0).astype(_BF16)
            return _dot(t, s_).astype(_BF16)

        qabs = [None] * NJ
        with _scope("I"):
            issue_ckv(2)
        with _scope("C_B2"):
            qabs[0] = absorb_j(0)
            qabs[2] = absorb_j(2)
        with _scope("I"):
            issue_ckv(3)
        with _scope("C_B2"):
            qabs[1] = absorb_j(1)
            qabs[3] = absorb_j(3)
            qabs = jnp.concatenate(qabs, axis=1)

        sc = [[None] * NU for _ in range(B)]

        def b_scores(u):
            for b in range(B):
                _wait_full(ckv_v.at[b, pl.ds(u * UR, UR)], csem.at[b, u])
                sc[b][u] = _dot_nt(qabs[b * H:(b + 1) * H], ckv_v[b, u * UR:(u + 1) * UR, :]) * scale

        def b_softmax(b):
            s = jnp.concatenate(sc[b], axis=1)
            m = jnp.max(s, axis=-1, keepdims=True)
            p = jnp.exp(s - m)
            l = jnp.sum(p, axis=-1, keepdims=True)
            return p.astype(_BF16), l

        def b_ctx(b, p, l):
            cc = _dot(p, ckv_v[b])
            return (cc / l).astype(_BF16)

        with _scope("I"):
            issue_ckv(4)
        with _scope("C_QK"):
            b_scores(0)
            b_scores(1)
        with _scope("I"):
            issue_ckv(5)
        with _scope("C_QK"):
            b_scores(2)
        with _scope("I"):
            issue_ckv(6)
        with _scope("C_QK"):
            b_scores(3)
        with _scope("I"):
            issue_ckv(7)
        with _scope("C_QK"):
            b_scores(4)
        with _scope("I"):
            issue_w3(2, wuv_hbm, wuv_v, 0)
        with _scope("C_QK"):
            b_scores(5)
        with _scope("I"):
            issue_w3(2, wuv_hbm, wuv_v, 1)
        with _scope("C_QK"):
            b_scores(6)
        with _scope("I"):
            issue_w512(wob_hbm, wob_v, sem.at[4], 0)
        with _scope("C_QK"):
            b_scores(7)
            p0, l0 = b_softmax(0)
        with _scope("I"):
            issue_w512(wob_hbm, wob_v, sem.at[4], 1)
        with _scope("C_PV"):
            p1, l1 = b_softmax(1)
            cc0 = b_ctx(0, p0, l0)
        with _scope("I"):
            issue_wq(0)
        with _scope("C_PV"):
            cc1 = b_ctx(1, p1, l1)
            ctxc = jnp.concatenate([cc0, cc1], axis=0)
        with _scope("I"):
            issue_wq(1)
        with _scope("C_B4"):
            ctx = project_j(ctxc, 2, wuv_v, 0) + project_j(ctxc, 2, wuv_v, 2)
        with _scope("I"):
            issue_w512(wo_hbm, wo_v, sem.at[5], 0)
            issue_w512(wo_hbm, wo_v, sem.at[5], 1)
        with _scope("C_B4"):
            ctx = ctx + project_j(ctxc, 2, wuv_v, 1) + project_j(ctxc, 2, wuv_v, 3)
        with _scope("I_kv0"):
            issue_kv(0, 0)
        with _scope("C_B5"):
            _wait_full(wob_v, sem.at[4])
            dmask = (jax.lax.broadcasted_iota(jnp.int32, (R, H * Dh), 1) // Dh
                     == jax.lax.broadcasted_iota(jnp.int32, (R, H * Dh), 0) % H)
            l2 = jnp.where(dmask, jnp.tile(ctx, (1, H)), 0.0).astype(_BF16)
            yb = _dot(l2, wob_v[...])
            outb = [jnp.sum(yb[b * H:(b + 1) * H], axis=0, keepdims=True) for b in range(B)]

            gw = gw_v[...].astype(_F32).reshape(1, D)
            xav = xa_v[...].astype(_F32)
            gate = jax.nn.sigmoid(jnp.sum(xav * gw, axis=-1, keepdims=True))
            base = (1.0 - gate) * jnp.concatenate(outb, axis=0)

        with _scope("C_QA"):
            _wait_full(wq_v, sem.at[3])
            xa = jnp.concatenate(
                [jnp.broadcast_to(xav[b:b + 1], (8, D)) for b in range(B)], axis=0).astype(_BF16)
            qa = _dot(xa, wq_v[...])
            for b in range(B):
                for h in range(H):
                    q_s[b * H + h] = qa[b * 8:(b + 1) * 8, h * Dh:(h + 1) * Dh].astype(_BF16)
            acc_s[...] = jnp.zeros_like(acc_s)
        with _scope("I_kv1"):
            for i in range(1, NSLOT - 1):
                issue_kv(i, i)
            _wait_full(wo_v, sem.at[5])

        def probs(i, slot):
            _wait_full(kbuf.at[slot], ksem.at[slot])
            s = _dot_nt(q_s[i], kbuf[slot]) * scale
            m = jnp.max(s, axis=-1, keepdims=True)
            p = jnp.exp(s - m)
            l = jnp.sum(p, axis=-1, keepdims=True)
            return p.astype(_BF16), l

        def step(i, carry):
            slot = i % NSLOT
            b = i // H
            h = i % H
            nxt = i + NSLOT - 1

            with _scope("I_kv"):
                @pl.when(nxt < BH - 1)
                def _():
                    issue_kv(nxt, nxt % NSLOT)

                @pl.when(nxt == BH - 1)
                def _():
                    issue_kv_last(BH - 1, (BH - 1) % NSLOT)

            with _scope("C_A"):
                p, l = probs(i, slot)
                _wait_full(vbuf.at[slot], vsem.at[slot])
                o = _dot(p, vbuf[slot]) / l
                y = _dot(o.astype(_BF16), wo_v[pl.ds(pl.multiple_of(h * Dh, Dh), Dh), :])
                acc_s[b] = acc_s[b] + y
            return carry

        jax.lax.fori_loop(0, BH - 1, step, 0)

        with _scope("C_last"):
            i = BH - 1
            slot = i % NSLOT
            p, l = probs(i, slot)
            o = jnp.zeros((8, Dh), _F32)
            for pc in range(VPIECES):
                r0 = pc * PR
                _wait_full(vbuf.at[slot, pl.ds(r0, PR)], lsem.at[pc])
                o = o + _dot(p[:, r0:r0 + PR], vbuf[slot, r0:r0 + PR, :])
            o = o / l
            y = _dot(o.astype(_BF16), wo_v[(H - 1) * Dh:H * Dh, :])
            a0 = acc_s[0][0:1]
            a1 = acc_s[1][0:1] + y[0:1]
            a = jnp.concatenate([a0, a1], axis=0)
            out_v[...] = (gate * a + base).astype(out_v.dtype)
            c_out = pltpu.make_async_copy(out_v, out_hbm, osem.at[0])
            c_out.start()
            c_out.wait()

    any_spec = pl.BlockSpec(memory_space=pl.ANY)
    bf = _BF16
    out = pl.pallas_call(
        kernel,
        in_specs=[any_spec] * 12,
        out_specs=any_spec,
        out_shape=jax.ShapeDtypeStruct((B, D), A_x.dtype),
        scratch_shapes=[
            pltpu.VMEM((B, D), bf),
            pltpu.VMEM((B, M), bf),
            pltpu.VMEM((D,), bf),
            pltpu.VMEM((D, H * Dh), bf),
            pltpu.VMEM((H * Dh, D), bf),
            pltpu.VMEM((B, Sk, Dc), bf),
            pltpu.VMEM((M * H, Dh), bf),
            pltpu.VMEM((Dc * H, Dh), bf),
            pltpu.VMEM((Dc * H, Dh), bf),
            pltpu.VMEM((H * Dh, M), bf),
            pltpu.VMEM((NSLOT, Sk, Dh), bf),
            pltpu.VMEM((NSLOT, Sk, Dh), bf),
            pltpu.VMEM((BH, 8, Dh), bf),
            pltpu.VMEM((B, 8, D), _F32),
            pltpu.VMEM((B, D), bf),
            pltpu.SemaphoreType.DMA((6,)),
            pltpu.SemaphoreType.DMA((3, NJ)),
            pltpu.SemaphoreType.DMA((B, NU)),
            pltpu.SemaphoreType.DMA((NSLOT,)),
            pltpu.SemaphoreType.DMA((NSLOT,)),
            pltpu.SemaphoreType.DMA((VPIECES,)),
            pltpu.SemaphoreType.DMA((1,)),
        ],
        compiler_params=pltpu.CompilerParams(vmem_limit_bytes=110 * 1024 * 1024,
                                             disable_semaphore_checks=True),
    )(xa2, xb2, gate_w, k3, v3, A_wq, A_wo, B_c_kv, wqb2, wuk2, wuv2, wob2)
    return out.reshape(B, Sq, D)
```

```python
import jax
import jax.numpy as jnp
import jax.experimental.pallas as pl
import jax.experimental.pallas.tpu as pltpu

_NT = (((1,), (1,)), ((), ()))
_F32 = jnp.float32
_BF16 = jnp.bfloat16

NSLOT = 3
SUB128 = 192
SUB512 = 48
ROFF = 26
VPIECES = 4


def _dot(a, b):
    return jnp.dot(a, b, preferred_element_type=_F32)


def _dot_nt(a, b):
    return jax.lax.dot_general(a, b, _NT, preferred_element_type=_F32)


def _stream2(src0, dst0, o0, sem0, src1, dst1, o1, sem1, rows, sub, rot=0):
    nfull = rows // sub
    rem = rows - nfull * sub

    def pair(off0, off1, n):
        pltpu.make_async_copy(src0.at[pl.ds(o0 + off0, n)], dst0.at[pl.ds(o0 + off0, n)],
                              sem0).start(priority=0)
        pltpu.make_async_copy(src1.at[pl.ds(o1 + off1, n)], dst1.at[pl.ds(o1 + off1, n)],
                              sem1).start(priority=1)

    def one(s, c):
        s1 = s
        if rot:
            s1 = jnp.where(s + rot >= nfull, s + rot - nfull, s + rot)
        pair(pl.multiple_of(s * sub, 16), pl.multiple_of(s1 * sub, 16), sub)
        return c

    jax.lax.fori_loop(0, nfull, one, 0, unroll=3)
    if rem:
        pair(nfull * sub, nfull * sub, rem)


def _wait_full(buf, sem):
    pltpu.make_async_copy(buf, buf, sem).wait()


@jax.jit
def pallas_gated_mix__mha_block_cached__compressed_kv_cla__decode_kernel(
    A_x: jax.Array,
    A_k_cache: jax.Array,
    A_v_cache: jax.Array,
    A_wq: jax.Array,
    A_wo: jax.Array,
    B_x: jax.Array,
    B_c_kv: jax.Array,
    B_w_q: jax.Array,
    B_w_uk: jax.Array,
    B_w_uv: jax.Array,
    B_w_o: jax.Array,
    gate_w: jax.Array,
):
    B, Sq, D = A_x.shape
    _, H, Sk, Dh = A_k_cache.shape
    Dc = B_c_kv.shape[-1]
    M = B_x.shape[-1]
    assert Sq == 1 and B == 2 and Dh == 128 and H == 32 and D == 512 and M == 512 and Dc == 512
    BH = B * H
    R = BH
    NJ = Dc // 128
    CH = 128 * H
    scale = float(Dh) ** -0.5
    NU = 8
    UR = Sk // NU
    PR = Sk // VPIECES

    xa2 = A_x.reshape(B, D)
    xb2 = B_x.reshape(B, M)
    k3 = A_k_cache.reshape(BH, Sk, Dh)
    v3 = A_v_cache.reshape(BH, Sk, Dh)
    wqb2 = B_w_q.reshape(M * H, Dh)
    wuk2 = B_w_uk.reshape(Dc * H, Dh)
    wuv2 = B_w_uv.reshape(Dc * H, Dh)
    wob2 = B_w_o.reshape(H * Dh, M)

    def kernel(xa_hbm, xb_hbm, gw_hbm, k_hbm, v_hbm, wq_hbm, wo_hbm, ckv_hbm,
               wqb_hbm, wuk_hbm, wuv_hbm, wob_hbm,
               out_hbm,
               xa_v, xb_v, gw_v, wq_v, wo_v, ckv_v, wqb_v, wuk_v, wuv_v, wob_v,
               kbuf, vbuf, q_s, acc_s, out_v,
               sem, jsem, csem, ksem, vsem, lsem, osem):

        def issue_w3(a, src, dst, u):
            _stream2(src, dst, u * CH, jsem.at[a, u],
                     src, dst, (u + 2) * CH, jsem.at[a, u + 2], CH, SUB128)

        def issue_ckv(u):
            _stream2(ckv_hbm.at[0], ckv_v.at[0], u * UR, csem.at[0, u],
                     ckv_hbm.at[1], ckv_v.at[1], u * UR, csem.at[1, u], UR, SUB512)

        def issue_w512(src, dst, s, u):
            qr = (H * Dh) // 4
            _stream2(src, dst, u * qr, s, src, dst, (u + 2) * qr, s, qr, SUB512)

        def issue_wq(u):
            qr = D // 4

            def one(s, c):
                r = pl.multiple_of(u * qr + s * 16, 16)
                r2 = pl.multiple_of(r + 2 * qr, 16)
                for col, n in ((0, 1408), (1408, 1408), (2816, 1280)):
                    pltpu.make_async_copy(wq_hbm.at[pl.ds(r, 16), pl.ds(col, n)],
                                          wq_v.at[pl.ds(r, 16), pl.ds(col, n)],
                                          sem.at[3]).start(priority=0)
                    pltpu.make_async_copy(wq_hbm.at[pl.ds(r2, 16), pl.ds(col, n)],
                                          wq_v.at[pl.ds(r2, 16), pl.ds(col, n)],
                                          sem.at[3]).start(priority=1)
                return c

            jax.lax.fori_loop(0, qr // 16, one, 0)

        def issue_kv(i, slot):
            _stream2(k_hbm.at[i], kbuf.at[slot], 0, ksem.at[slot],
                     v_hbm.at[i], vbuf.at[slot], 0, vsem.at[slot], Sk, SUB128, rot=ROFF)

        def issue_kv_last(i, slot):
            for p in range(VPIECES):
                _stream2(k_hbm.at[i], kbuf.at[slot], p * PR, ksem.at[slot],
                         v_hbm.at[i], vbuf.at[slot], p * PR, lsem.at[p], PR, SUB128)

        def wait_w3(a, ref, j):
            _wait_full(ref.at[pl.ds(j * CH, CH)], jsem.at[a, j])

        c_xa = pltpu.make_async_copy(xa_hbm, xa_v, sem.at[0])
        c_xb = pltpu.make_async_copy(xb_hbm, xb_v, sem.at[1])
        c_gw = pltpu.make_async_copy(gw_hbm, gw_v, sem.at[2])
        issue_w3(0, wqb_hbm, wqb_v, 0)
        c_xb.start()
        c_xa.start()
        c_gw.start()
        issue_w3(0, wqb_hbm, wqb_v, 1)
        issue_w3(1, wuk_hbm, wuk_v, 0)

        st = (jax.lax.broadcasted_iota(jnp.int32, (128, CH), 1) // H
              == jax.lax.broadcasted_iota(jnp.int32, (128, CH), 0)).astype(_F32).astype(_BF16)
        s_ = (jax.lax.broadcasted_iota(jnp.int32, (CH, 128), 0) // H
              == jax.lax.broadcasted_iota(jnp.int32, (CH, 128), 1)).astype(_F32).astype(_BF16)
        hmask = (jax.lax.broadcasted_iota(jnp.int32, (R, CH), 1) % H
                 == jax.lax.broadcasted_iota(jnp.int32, (R, CH), 0) % H)

        def project_j(c, a, w_ref, j):
            e = _dot(c[:, j * 128:(j + 1) * 128], st)
            l = jnp.where(hmask, e, 0.0).astype(_BF16)
            wait_w3(a, w_ref, j)
            return _dot(l, w_ref[j * CH:(j + 1) * CH, :])

        issue_w3(1, wuk_hbm, wuk_v, 1)
        issue_ckv(0)
        c_xb.wait()
        c_xa.wait()
        c_gw.wait()
        xbv = xb_v[...].astype(_F32)
        xb = jnp.concatenate(
            [jnp.broadcast_to(xbv[b:b + 1], (H, M)) for b in range(B)], axis=0).astype(_BF16)
        qb = project_j(xb, 0, wqb_v, 0) + project_j(xb, 0, wqb_v, 2)
        issue_ckv(1)
        qb = qb + project_j(xb, 0, wqb_v, 1) + project_j(xb, 0, wqb_v, 3)
        qb = qb.astype(_BF16)

        def absorb_j(j):
            wait_w3(1, wuk_v, j)
            t = _dot_nt(qb, wuk_v[j * CH:(j + 1) * CH, :])
            t = jnp.where(hmask, t, 0.0).astype(_BF16)
            return _dot(t, s_).astype(_BF16)

        qabs = [None] * NJ
        issue_ckv(2)
        qabs[0] = absorb_j(0)
        qabs[2] = absorb_j(2)
        issue_ckv(3)
        qabs[1] = absorb_j(1)
        qabs[3] = absorb_j(3)
        qabs = jnp.concatenate(qabs, axis=1)

        sc = [[None] * NU for _ in range(B)]

        def b_scores(u):
            for b in range(B):
                _wait_full(ckv_v.at[b, pl.ds(u * UR, UR)], csem.at[b, u])
                sc[b][u] = _dot_nt(qabs[b * H:(b + 1) * H],
                                   ckv_v[b, u * UR:(u + 1) * UR, :]) * scale

        def b_softmax(b):
            s = jnp.concatenate(sc[b], axis=1)
            m = jnp.max(s, axis=-1, keepdims=True)
            p = jnp.exp(s - m)
            l = jnp.sum(p, axis=-1, keepdims=True)
            return p.astype(_BF16), l

        def b_ctx(b, p, l):
            cc = _dot(p, ckv_v[b])
            return (cc / l).astype(_BF16)

        issue_ckv(4)
        b_scores(0)
        b_scores(1)
        issue_ckv(5)
        b_scores(2)
        issue_ckv(6)
        b_scores(3)
        issue_ckv(7)
        b_scores(4)
        issue_w3(2, wuv_hbm, wuv_v, 0)
        b_scores(5)
        issue_w3(2, wuv_hbm, wuv_v, 1)
        b_scores(6)
        issue_w512(wob_hbm, wob_v, sem.at[4], 0)
        b_scores(7)
        p0, l0 = b_softmax(0)
        issue_w512(wob_hbm, wob_v, sem.at[4], 1)
        p1, l1 = b_softmax(1)
        cc0 = b_ctx(0, p0, l0)
        issue_wq(0)
        cc1 = b_ctx(1, p1, l1)
        ctxc = jnp.concatenate([cc0, cc1], axis=0)
        issue_wq(1)
        ctx = project_j(ctxc, 2, wuv_v, 0) + project_j(ctxc, 2, wuv_v, 2)
        issue_w512(wo_hbm, wo_v, sem.at[5], 0)
        issue_w512(wo_hbm, wo_v, sem.at[5], 1)
        ctx = ctx + project_j(ctxc, 2, wuv_v, 1) + project_j(ctxc, 2, wuv_v, 3)
        issue_kv(0, 0)

        _wait_full(wob_v, sem.at[4])
        dmask = (jax.lax.broadcasted_iota(jnp.int32, (R, H * Dh), 1) // Dh
                 == jax.lax.broadcasted_iota(jnp.int32, (R, H * Dh), 0) % H)
        l2 = jnp.where(dmask, jnp.tile(ctx, (1, H)), 0.0).astype(_BF16)
        yb = _dot(l2, wob_v[...])
        outb = [jnp.sum(yb[b * H:(b + 1) * H], axis=0, keepdims=True) for b in range(B)]

        gw = gw_v[...].astype(_F32).reshape(1, D)
        xav = xa_v[...].astype(_F32)
        gate = jax.nn.sigmoid(jnp.sum(xav * gw, axis=-1, keepdims=True))
        base = (1.0 - gate) * jnp.concatenate(outb, axis=0)

        _wait_full(wq_v, sem.at[3])
        xa = jnp.concatenate(
            [jnp.broadcast_to(xav[b:b + 1], (8, D)) for b in range(B)], axis=0).astype(_BF16)
        qa = _dot(xa, wq_v[...])
        for b in range(B):
            for h in range(H):
                q_s[b * H + h] = qa[b * 8:(b + 1) * 8, h * Dh:(h + 1) * Dh].astype(_BF16)
        acc_s[...] = jnp.zeros_like(acc_s)
        for i in range(1, NSLOT - 1):
            issue_kv(i, i)
        _wait_full(wo_v, sem.at[5])

        def probs(i, slot):
            _wait_full(kbuf.at[slot], ksem.at[slot])
            s = _dot_nt(q_s[i], kbuf[slot]) * scale
            m = jnp.max(s, axis=-1, keepdims=True)
            p = jnp.exp(s - m)
            l = jnp.sum(p, axis=-1, keepdims=True)
            return p.astype(_BF16), l

        def step(i, carry):
            slot = i % NSLOT
            b = i // H
            h = i % H
            nxt = i + NSLOT - 1

            @pl.when(nxt < BH - 1)
            def _():
                issue_kv(nxt, nxt % NSLOT)

            @pl.when(nxt == BH - 1)
            def _():
                issue_kv_last(BH - 1, (BH - 1) % NSLOT)

            p, l = probs(i, slot)
            _wait_full(vbuf.at[slot], vsem.at[slot])
            o = _dot(p, vbuf[slot]) / l
            y = _dot(o.astype(_BF16), wo_v[pl.ds(pl.multiple_of(h * Dh, Dh), Dh), :])
            acc_s[b] = acc_s[b] + y
            return carry

        jax.lax.fori_loop(0, BH - 1, step, 0)

        i = BH - 1
        slot = i % NSLOT
        p, l = probs(i, slot)
        o = jnp.zeros((8, Dh), _F32)
        for pc in range(VPIECES):
            r0 = pc * PR
            _wait_full(vbuf.at[slot, pl.ds(r0, PR)], lsem.at[pc])
            o = o + _dot(p[:, r0:r0 + PR], vbuf[slot, r0:r0 + PR, :])
        o = o / l
        y = _dot(o.astype(_BF16), wo_v[(H - 1) * Dh:H * Dh, :])
        a = jnp.concatenate([acc_s[0][0:1], acc_s[1][0:1] + y[0:1]], axis=0)
        out_v[...] = (gate * a + base).astype(out_v.dtype)
        c_out = pltpu.make_async_copy(out_v, out_hbm, osem.at[0])
        c_out.start()
        c_out.wait()

    any_spec = pl.BlockSpec(memory_space=pl.ANY)
    bf = _BF16
    out = pl.pallas_call(
        kernel,
        in_specs=[any_spec] * 12,
        out_specs=any_spec,
        out_shape=jax.ShapeDtypeStruct((B, D), A_x.dtype),
        scratch_shapes=[
            pltpu.VMEM((B, D), bf),
            pltpu.VMEM((B, M), bf),
            pltpu.VMEM((D,), bf),
            pltpu.VMEM((D, H * Dh), bf),
            pltpu.VMEM((H * Dh, D), bf),
            pltpu.VMEM((B, Sk, Dc), bf),
            pltpu.VMEM((M * H, Dh), bf),
            pltpu.VMEM((Dc * H, Dh), bf),
            pltpu.VMEM((Dc * H, Dh), bf),
            pltpu.VMEM((H * Dh, M), bf),
            pltpu.VMEM((NSLOT, Sk, Dh), bf),
            pltpu.VMEM((NSLOT, Sk, Dh), bf),
            pltpu.VMEM((BH, 8, Dh), bf),
            pltpu.VMEM((B, 8, D), _F32),
            pltpu.VMEM((B, D), bf),
            pltpu.SemaphoreType.DMA((6,)),
            pltpu.SemaphoreType.DMA((3, NJ)),
            pltpu.SemaphoreType.DMA((B, NU)),
            pltpu.SemaphoreType.DMA((NSLOT,)),
            pltpu.SemaphoreType.DMA((NSLOT,)),
            pltpu.SemaphoreType.DMA((VPIECES,)),
            pltpu.SemaphoreType.DMA((1,)),
        ],
        compiler_params=pltpu.CompilerParams(vmem_limit_bytes=110 * 1024 * 1024,
                                             disable_semaphore_checks=True),
    )(xa2, xb2, gate_w, k3, v3, A_wq, A_wo, B_c_kv, wqb2, wuk2, wuv2, wob2)
    return out.reshape(B, Sq, D)
```

```python
import jax
import jax.numpy as jnp
import jax.experimental.pallas as pl
import jax.experimental.pallas.tpu as pltpu

_NT = (((1,), (1,)), ((), ()))
_F32 = jnp.float32
_BF16 = jnp.bfloat16

NSLOT = 3
SUB128 = 192
SUB512 = 48
ROFF = 26
VPIECES = 4


def _dot(a, b):
    return jnp.dot(a, b, preferred_element_type=_F32)


def _dot_nt(a, b):
    return jax.lax.dot_general(a, b, _NT, preferred_element_type=_F32)


def _stream2(src0, dst0, o0, sem0, src1, dst1, o1, sem1, rows, sub, rot=0):
    nfull = rows // sub
    rem = rows - nfull * sub
    rot = rot % nfull

    def pair(off0, off1, n):
        pltpu.make_async_copy(src0.at[pl.ds(o0 + off0, n)], dst0.at[pl.ds(o0 + off0, n)],
                              sem0).start(priority=0)
        pltpu.make_async_copy(src1.at[pl.ds(o1 + off1, n)], dst1.at[pl.ds(o1 + off1, n)],
                              sem1).start(priority=1)

    def one(s, c):
        s1 = s
        if rot:
            s1 = jnp.where(s + rot >= nfull, s + rot - nfull, s + rot)
        pair(pl.multiple_of(s * sub, 16), pl.multiple_of(s1 * sub, 16), sub)
        return c

    jax.lax.fori_loop(0, nfull, one, 0, unroll=3)
    if rem:
        pair(nfull * sub, nfull * sub, rem)


def _wait_full(buf, sem):
    pltpu.make_async_copy(buf, buf, sem).wait()


@jax.jit
def pallas_gated_mix__mha_block_cached__compressed_kv_cla__decode_kernel(
    A_x: jax.Array,
    A_k_cache: jax.Array,
    A_v_cache: jax.Array,
    A_wq: jax.Array,
    A_wo: jax.Array,
    B_x: jax.Array,
    B_c_kv: jax.Array,
    B_w_q: jax.Array,
    B_w_uk: jax.Array,
    B_w_uv: jax.Array,
    B_w_o: jax.Array,
    gate_w: jax.Array,
):
    B, Sq, D = A_x.shape
    _, H, Sk, Dh = A_k_cache.shape
    Dc = B_c_kv.shape[-1]
    M = B_w_q.shape[0]
    assert Sq == 1 and B == 2 and Dh == 128 and H == 32 and D == 512 and M == D and Dc == 512
    BH = B * H
    R = BH
    NJ = Dc // 128
    CH = 128 * H
    scale = float(Dh) ** -0.5
    NU = 8
    UR = Sk // NU
    PR = Sk // VPIECES

    xa2 = A_x.reshape(B, D)
    k3 = A_k_cache.reshape(BH, Sk, Dh)
    v3 = A_v_cache.reshape(BH, Sk, Dh)
    wqb2 = B_w_q.reshape(M * H, Dh)
    wuk2 = B_w_uk.reshape(Dc * H, Dh)
    wuv2 = B_w_uv.reshape(Dc * H, Dh)
    wob2 = B_w_o.reshape(H * Dh, M)

    def kernel(xa_hbm, gw_hbm, k_hbm, v_hbm, wq_hbm, wo_hbm, ckv_hbm,
               wqb_hbm, wuk_hbm, wuv_hbm, wob_hbm,
               out_hbm,
               xa_v, gw_v, wq_v, wo_v, ckv_v, wqb_v, wuk_v, wuv_v, wob_v,
               kbuf, vbuf, q_s, acc_s, out_v,
               sem, jsem, csem, ksem, vsem, lsem, osem):

        def issue_w3(a, src, dst, u):
            _stream2(src, dst, u * CH, jsem.at[a, u],
                     src, dst, (u + 2) * CH, jsem.at[a, u + 2], CH, SUB128)

        def issue_ckv(u):
            _stream2(ckv_hbm.at[0], ckv_v.at[0], u * UR, csem.at[0, u],
                     ckv_hbm.at[1], ckv_v.at[1], u * UR, csem.at[1, u], UR, SUB512)

        def issue_w512(src, dst, s, u):
            qr = (H * Dh) // 4
            _stream2(src, dst, u * qr, s, src, dst, (u + 2) * qr, s, qr, SUB512)

        def issue_wq(u):
            qr = D // 4

            def one(s, c):
                r = pl.multiple_of(u * qr + s * 16, 16)
                r2 = pl.multiple_of(r + 2 * qr, 16)
                for col, n in ((0, 1408), (1408, 1408), (2816, 1280)):
                    pltpu.make_async_copy(wq_hbm.at[pl.ds(r, 16), pl.ds(col, n)],
                                          wq_v.at[pl.ds(r, 16), pl.ds(col, n)],
                                          sem.at[2]).start(priority=0)
                    pltpu.make_async_copy(wq_hbm.at[pl.ds(r2, 16), pl.ds(col, n)],
                                          wq_v.at[pl.ds(r2, 16), pl.ds(col, n)],
                                          sem.at[2]).start(priority=1)
                return c

            jax.lax.fori_loop(0, qr // 16, one, 0)

        def issue_kv(i, slot):
            _stream2(k_hbm.at[i], kbuf.at[slot], 0, ksem.at[slot],
                     v_hbm.at[i], vbuf.at[slot], 0, vsem.at[slot], Sk, SUB128, rot=ROFF)

        def issue_kv_last(i, slot):
            for p in range(VPIECES):
                _stream2(k_hbm.at[i], kbuf.at[slot], p * PR, ksem.at[slot],
                         v_hbm.at[i], vbuf.at[slot], p * PR, lsem.at[p], PR, SUB128)

        def wait_w3(a, ref, j):
            _wait_full(ref.at[pl.ds(j * CH, CH)], jsem.at[a, j])

        c_xa = pltpu.make_async_copy(xa_hbm, xa_v, sem.at[0])
        c_gw = pltpu.make_async_copy(gw_hbm, gw_v, sem.at[1])
        issue_w3(0, wqb_hbm, wqb_v, 0)
        c_xa.start()
        c_gw.start()
        issue_w3(0, wqb_hbm, wqb_v, 1)
        issue_w3(1, wuk_hbm, wuk_v, 0)

        st = (jax.lax.broadcasted_iota(jnp.int32, (128, CH), 1) // H
              == jax.lax.broadcasted_iota(jnp.int32, (128, CH), 0)).astype(_F32).astype(_BF16)
        s_ = (jax.lax.broadcasted_iota(jnp.int32, (CH, 128), 0) // H
              == jax.lax.broadcasted_iota(jnp.int32, (CH, 128), 1)).astype(_F32).astype(_BF16)
        hmask = (jax.lax.broadcasted_iota(jnp.int32, (R, CH), 1) % H
                 == jax.lax.broadcasted_iota(jnp.int32, (R, CH), 0) % H)

        def project_j(c, a, w_ref, j):
            e = _dot(c[:, j * 128:(j + 1) * 128], st)
            l = jnp.where(hmask, e, 0.0).astype(_BF16)
            wait_w3(a, w_ref, j)
            return _dot(l, w_ref[j * CH:(j + 1) * CH, :])

        issue_w3(1, wuk_hbm, wuk_v, 1)
        issue_ckv(0)
        c_xa.wait()
        c_gw.wait()
        xav = xa_v[...].astype(_F32)
        xb = jnp.concatenate(
            [jnp.broadcast_to(xav[b:b + 1], (H, M)) for b in range(B)], axis=0).astype(_BF16)
        qb = project_j(xb, 0, wqb_v, 0) + project_j(xb, 0, wqb_v, 2)
        issue_ckv(1)
        qb = qb + project_j(xb, 0, wqb_v, 1) + project_j(xb, 0, wqb_v, 3)
        qb = qb.astype(_BF16)

        def absorb_j(j):
            wait_w3(1, wuk_v, j)
            t = _dot_nt(qb, wuk_v[j * CH:(j + 1) * CH, :])
            t = jnp.where(hmask, t, 0.0).astype(_BF16)
            return _dot(t, s_).astype(_BF16)

        qabs = [None] * NJ
        issue_ckv(2)
        qabs[0] = absorb_j(0)
        qabs[2] = absorb_j(2)
        issue_ckv(3)
        qabs[1] = absorb_j(1)
        qabs[3] = absorb_j(3)
        qabs = jnp.concatenate(qabs, axis=1)

        sc = [[None] * NU for _ in range(B)]

        def b_scores(u):
            for b in range(B):
                _wait_full(ckv_v.at[b, pl.ds(u * UR, UR)], csem.at[b, u])
                sc[b][u] = _dot_nt(qabs[b * H:(b + 1) * H],
                                   ckv_v[b, u * UR:(u + 1) * UR, :]) * scale

        def b_softmax(b):
            s = jnp.concatenate(sc[b], axis=1)
            m = jnp.max(s, axis=-1, keepdims=True)
            p = jnp.exp(s - m)
            l = jnp.sum(p, axis=-1, keepdims=True)
            return p.astype(_BF16), l

        def b_ctx(b, p, l):
            cc = _dot(p, ckv_v[b])
            return (cc / l).astype(_BF16)

        issue_ckv(4)
        b_scores(0)
        b_scores(1)
        issue_ckv(5)
        b_scores(2)
        issue_ckv(6)
        b_scores(3)
        issue_ckv(7)
        b_scores(4)
        issue_w3(2, wuv_hbm, wuv_v, 0)
        b_scores(5)
        issue_w3(2, wuv_hbm, wuv_v, 1)
        b_scores(6)
        issue_w512(wob_hbm, wob_v, sem.at[3], 0)
        b_scores(7)
        p0, l0 = b_softmax(0)
        issue_w512(wob_hbm, wob_v, sem.at[3], 1)
        p1, l1 = b_softmax(1)
        cc0 = b_ctx(0, p0, l0)
        issue_wq(0)
        cc1 = b_ctx(1, p1, l1)
        ctxc = jnp.concatenate([cc0, cc1], axis=0)
        issue_wq(1)
        ctx = project_j(ctxc, 2, wuv_v, 0) + project_j(ctxc, 2, wuv_v, 2)
        issue_w512(wo_hbm, wo_v, sem.at[4], 0)
        issue_w512(wo_hbm, wo_v, sem.at[4], 1)
        ctx = ctx + project_j(ctxc, 2, wuv_v, 1) + project_j(ctxc, 2, wuv_v, 3)
        issue_kv(0, 0)

        _wait_full(wob_v, sem.at[3])
        dmask = (jax.lax.broadcasted_iota(jnp.int32, (R, H * Dh), 1) // Dh
                 == jax.lax.broadcasted_iota(jnp.int32, (R, H * Dh), 0) % H)
        l2 = jnp.where(dmask, jnp.tile(ctx, (1, H)), 0.0).astype(_BF16)
        yb = _dot(l2, wob_v[...])
        outb = [jnp.sum(yb[b * H:(b + 1) * H], axis=0, keepdims=True) for b in range(B)]

        gw = gw_v[...].astype(_F32).reshape(1, D)
        gate = jax.nn.sigmoid(jnp.sum(xav * gw, axis=-1, keepdims=True))
        base = (1.0 - gate) * jnp.concatenate(outb, axis=0)

        _wait_full(wq_v, sem.at[2])
        xa = jnp.concatenate(
            [jnp.broadcast_to(xav[b:b + 1], (8, D)) for b in range(B)], axis=0).astype(_BF16)
        qa = _dot(xa, wq_v[...])
        for b in range(B):
            for h in range(H):
                q_s[b * H + h] = qa[b * 8:(b + 1) * 8, h * Dh:(h + 1) * Dh].astype(_BF16)
        acc_s[...] = jnp.zeros_like(acc_s)
        for i in range(1, NSLOT - 1):
            issue_kv(i, i)
        _wait_full(wo_v, sem.at[4])

        def probs(i, slot):
            _wait_full(kbuf.at[slot], ksem.at[slot])
            s = _dot_nt(q_s[i], kbuf[slot]) * scale
            m = jnp.max(s, axis=-1, keepdims=True)
            p = jnp.exp(s - m)
            l = jnp.sum(p, axis=-1, keepdims=True)
            return p.astype(_BF16), l

        def step(i, carry):
            slot = i % NSLOT
            b = i // H
            h = i % H
            nxt = i + NSLOT - 1

            @pl.when(nxt < BH - 1)
            def _():
                issue_kv(nxt, nxt % NSLOT)

            @pl.when(nxt == BH - 1)
            def _():
                issue_kv_last(BH - 1, (BH - 1) % NSLOT)

            p, l = probs(i, slot)
            _wait_full(vbuf.at[slot], vsem.at[slot])
            o = _dot(p, vbuf[slot]) / l
            y = _dot(o.astype(_BF16), wo_v[pl.ds(pl.multiple_of(h * Dh, Dh), Dh), :])
            acc_s[b] = acc_s[b] + y
            return carry

        jax.lax.fori_loop(0, BH - 1, step, 0)

        i = BH - 1
        slot = i % NSLOT
        p, l = probs(i, slot)
        o = jnp.zeros((8, Dh), _F32)
        for pc in range(VPIECES):
            r0 = pc * PR
            _wait_full(vbuf.at[slot, pl.ds(r0, PR)], lsem.at[pc])
            o = o + _dot(p[:, r0:r0 + PR], vbuf[slot, r0:r0 + PR, :])
        o = o / l
        y = _dot(o.astype(_BF16), wo_v[(H - 1) * Dh:H * Dh, :])
        a = jnp.concatenate([acc_s[0][0:1], acc_s[1][0:1] + y[0:1]], axis=0)
        out_v[...] = (gate * a + base).astype(out_v.dtype)
        c_out = pltpu.make_async_copy(out_v, out_hbm, osem.at[0])
        c_out.start()
        c_out.wait()

    any_spec = pl.BlockSpec(memory_space=pl.ANY)
    bf = _BF16
    out = pl.pallas_call(
        kernel,
        in_specs=[any_spec] * 11,
        out_specs=any_spec,
        out_shape=jax.ShapeDtypeStruct((B, D), A_x.dtype),
        scratch_shapes=[
            pltpu.VMEM((B, D), bf),
            pltpu.VMEM((D,), bf),
            pltpu.VMEM((D, H * Dh), bf),
            pltpu.VMEM((H * Dh, D), bf),
            pltpu.VMEM((B, Sk, Dc), bf),
            pltpu.VMEM((M * H, Dh), bf),
            pltpu.VMEM((Dc * H, Dh), bf),
            pltpu.VMEM((Dc * H, Dh), bf),
            pltpu.VMEM((H * Dh, M), bf),
            pltpu.VMEM((NSLOT, Sk, Dh), bf),
            pltpu.VMEM((NSLOT, Sk, Dh), bf),
            pltpu.VMEM((BH, 8, Dh), bf),
            pltpu.VMEM((B, 8, D), _F32),
            pltpu.VMEM((B, D), bf),
            pltpu.SemaphoreType.DMA((5,)),
            pltpu.SemaphoreType.DMA((3, NJ)),
            pltpu.SemaphoreType.DMA((B, NU)),
            pltpu.SemaphoreType.DMA((NSLOT,)),
            pltpu.SemaphoreType.DMA((NSLOT,)),
            pltpu.SemaphoreType.DMA((VPIECES,)),
            pltpu.SemaphoreType.DMA((1,)),
        ],
        compiler_params=pltpu.CompilerParams(vmem_limit_bytes=110 * 1024 * 1024,
                                             disable_semaphore_checks=True),
    )(xa2, gate_w, k3, v3, A_wq, A_wo, B_c_kv, wqb2, wuk2, wuv2, wob2)
    return out.reshape(B, Sq, D)
```

```python
import jax
import jax.numpy as jnp
import jax.experimental.pallas as pl
import jax.experimental.pallas.tpu as pltpu

_NT = (((1,), (1,)), ((), ()))
_F32 = jnp.float32
_BF16 = jnp.bfloat16

NSLOT = 2
HPC = 4
NBLK = 2 * HPC
KVSUB = 16
LSUB = 96
NPART = 2
SUB128 = 192
SUB512 = 48
VPIECES = 4


def _dot(a, b):
    return jnp.dot(a, b, preferred_element_type=_F32)


def _dot_nt(a, b):
    return jax.lax.dot_general(a, b, _NT, preferred_element_type=_F32)


def _stream2(src0, dst0, o0, sem0, src1, dst1, o1, sem1, rows, sub, rot=0):
    nfull = rows // sub
    rem = rows - nfull * sub
    rot = rot % nfull

    def pair(off0, off1, n):
        pltpu.make_async_copy(src0.at[pl.ds(o0 + off0, n)], dst0.at[pl.ds(o0 + off0, n)],
                              sem0).start(priority=0)
        pltpu.make_async_copy(src1.at[pl.ds(o1 + off1, n)], dst1.at[pl.ds(o1 + off1, n)],
                              sem1).start(priority=1)

    def one(s, c):
        s1 = s
        if rot:
            s1 = jnp.where(s + rot >= nfull, s + rot - nfull, s + rot)
        pair(pl.multiple_of(s * sub, 16), pl.multiple_of(s1 * sub, 16), sub)
        return c

    jax.lax.fori_loop(0, nfull, one, 0, unroll=3)
    if rem:
        pair(nfull * sub, nfull * sub, rem)


def _wait_full(buf, sem):
    pltpu.make_async_copy(buf, buf, sem).wait()


@jax.jit
def pallas_gated_mix__mha_block_cached__compressed_kv_cla__decode_kernel(
    A_x: jax.Array,
    A_k_cache: jax.Array,
    A_v_cache: jax.Array,
    A_wq: jax.Array,
    A_wo: jax.Array,
    B_x: jax.Array,
    B_c_kv: jax.Array,
    B_w_q: jax.Array,
    B_w_uk: jax.Array,
    B_w_uv: jax.Array,
    B_w_o: jax.Array,
    gate_w: jax.Array,
):
    B, Sq, D = A_x.shape
    _, H, Sk, Dh = A_k_cache.shape
    Dc = B_c_kv.shape[-1]
    M = B_w_q.shape[0]
    assert Sq == 1 and B == 2 and Dh == 128 and H == 32 and D == 512 and M == D and Dc == 512
    BH = B * H
    R = BH
    NJ = Dc // 128
    CH = 128 * H
    scale = float(Dh) ** -0.5
    NU = 8
    UR = Sk // NU
    PR = (Sk // 2) // VPIECES

    xa2 = A_x.reshape(B, D)
    HS = Sk // 2
    NCH = BH // HPC
    k3 = A_k_cache.reshape(NCH, NBLK, HS, Dh)
    v3 = A_v_cache.reshape(NCH, NBLK, HS, Dh)
    wqb2 = B_w_q.reshape(M * H, Dh)
    wuk2 = B_w_uk.reshape(Dc * H, Dh)
    wuv2 = B_w_uv.reshape(Dc * H, Dh)
    wob2 = B_w_o.reshape(H * Dh, M)

    def kernel(xa_hbm, gw_hbm, k_hbm, v_hbm, wq_hbm, wo_hbm, ckv_hbm,
               wqb_hbm, wuk_hbm, wuv_hbm, wob_hbm,
               out_hbm,
               xa_v, gw_v, wq_v, wo_v, ckv_v, wqb_v, wuk_v, wuv_v, wob_v,
               kbuf, vbuf, q_s, acc_s, out_v,
               sem, jsem, csem, ksem, vsem, hsem, lsem, osem):

        def issue_w3(a, src, dst, u):
            _stream2(src, dst, u * CH, jsem.at[a, u],
                     src, dst, (u + 2) * CH, jsem.at[a, u + 2], CH, SUB128)

        def issue_ckv(u):
            _stream2(ckv_hbm.at[0], ckv_v.at[0], u * UR, csem.at[0, u],
                     ckv_hbm.at[1], ckv_v.at[1], u * UR, csem.at[1, u], UR, SUB512)

        def issue_w512(src, dst, s, u):
            qr = (H * Dh) // 4
            _stream2(src, dst, u * qr, s, src, dst, (u + 2) * qr, s, qr, SUB512)

        def issue_wq(u):
            qr = D // 4

            def one(s, c):
                r = pl.multiple_of(u * qr + s * 16, 16)
                r2 = pl.multiple_of(r + 2 * qr, 16)
                for col, n in ((0, 1408), (1408, 1408), (2816, 1280)):
                    pltpu.make_async_copy(wq_hbm.at[pl.ds(r, 16), pl.ds(col, n)],
                                          wq_v.at[pl.ds(r, 16), pl.ds(col, n)],
                                          sem.at[2]).start(priority=0)
                    pltpu.make_async_copy(wq_hbm.at[pl.ds(r2, 16), pl.ds(col, n)],
                                          wq_v.at[pl.ds(r2, 16), pl.ds(col, n)],
                                          sem.at[2]).start(priority=1)
                return c

            jax.lax.fori_loop(0, qr // 16, one, 0)

        def kv_pairs(ksrc, kdst, ks, vsrc, vdst, vs, r0, rows, sub):
            nfull = rows // sub
            rem = rows - nfull * sub

            def pair(off, n):
                pltpu.make_async_copy(ksrc.at[:, pl.ds(off, n)], kdst.at[:, pl.ds(off, n)], ks).start(priority=0)
                pltpu.make_async_copy(vsrc.at[:, pl.ds(off, n)], vdst.at[:, pl.ds(off, n)], vs).start(priority=1)

            def one(t, c):
                pair(pl.multiple_of(r0 + t * sub, 16), sub)
                return c

            jax.lax.fori_loop(0, nfull, one, 0, unroll=4)
            if rem:
                pair(r0 + nfull * sub, rem)

        NP = HPC * NPART
        PROWS = HS // NP

        def issue_chunk_part(c, part):
            slot = c % NSLOT
            kv_pairs(k_hbm.at[c], kbuf.at[slot], ksem.at[slot], v_hbm.at[c], vbuf.at[slot], vsem.at[slot],
                     part * PROWS, PROWS, KVSUB)

        LSLOT = (NCH - 1) % NSLOT

        def issue_last_part(hh, u):
            blk = pl.ds(2 * hh, 2)
            kv_pairs(k_hbm.at[NCH - 1, blk], kbuf.at[LSLOT, blk], hsem.at[0, hh],
                     v_hbm.at[NCH - 1, blk], vbuf.at[LSLOT, blk], hsem.at[1, hh],
                     u * (HS // NPART), HS // NPART, LSUB)

        def issue_last_head():
            hh = HPC - 1
            blk = pl.ds(2 * hh, 2)
            for p in range(VPIECES):
                kv_pairs(k_hbm.at[NCH - 1, blk], kbuf.at[LSLOT, blk], hsem.at[0, hh],
                         v_hbm.at[NCH - 1, blk], vbuf.at[LSLOT, blk], lsem.at[p], p * PR, PR, LSUB)

        def wait_w3(a, ref, j):
            _wait_full(ref.at[pl.ds(j * CH, CH)], jsem.at[a, j])

        c_xa = pltpu.make_async_copy(xa_hbm, xa_v, sem.at[0])
        c_gw = pltpu.make_async_copy(gw_hbm, gw_v, sem.at[1])
        issue_w3(0, wqb_hbm, wqb_v, 0)
        c_xa.start()
        c_gw.start()
        issue_w3(0, wqb_hbm, wqb_v, 1)
        issue_w3(1, wuk_hbm, wuk_v, 0)

        st = (jax.lax.broadcasted_iota(jnp.int32, (128, CH), 1) // H
              == jax.lax.broadcasted_iota(jnp.int32, (128, CH), 0)).astype(_F32).astype(_BF16)
        s_ = (jax.lax.broadcasted_iota(jnp.int32, (CH, 128), 0) // H
              == jax.lax.broadcasted_iota(jnp.int32, (CH, 128), 1)).astype(_F32).astype(_BF16)
        hmask = (jax.lax.broadcasted_iota(jnp.int32, (R, CH), 1) % H
                 == jax.lax.broadcasted_iota(jnp.int32, (R, CH), 0) % H)

        def project_j(c, a, w_ref, j):
            e = _dot(c[:, j * 128:(j + 1) * 128], st)
            l = jnp.where(hmask, e, 0.0).astype(_BF16)
            wait_w3(a, w_ref, j)
            return _dot(l, w_ref[j * CH:(j + 1) * CH, :])

        issue_w3(1, wuk_hbm, wuk_v, 1)
        issue_ckv(0)
        c_xa.wait()
        c_gw.wait()
        xav = xa_v[...].astype(_F32)
        xb = jnp.concatenate(
            [jnp.broadcast_to(xav[b:b + 1], (H, M)) for b in range(B)], axis=0).astype(_BF16)
        qb = project_j(xb, 0, wqb_v, 0) + project_j(xb, 0, wqb_v, 2)
        issue_ckv(1)
        qb = qb + project_j(xb, 0, wqb_v, 1) + project_j(xb, 0, wqb_v, 3)
        qb = qb.astype(_BF16)

        def absorb_j(j):
            wait_w3(1, wuk_v, j)
            t = _dot_nt(qb, wuk_v[j * CH:(j + 1) * CH, :])
            t = jnp.where(hmask, t, 0.0).astype(_BF16)
            return _dot(t, s_).astype(_BF16)

        qabs = [None] * NJ
        issue_ckv(2)
        qabs[0] = absorb_j(0)
        qabs[2] = absorb_j(2)
        issue_ckv(3)
        qabs[1] = absorb_j(1)
        qabs[3] = absorb_j(3)
        qabs = jnp.concatenate(qabs, axis=1)

        sc = [[None] * NU for _ in range(B)]

        def b_scores(u):
            for b in range(B):
                _wait_full(ckv_v.at[b, pl.ds(u * UR, UR)], csem.at[b, u])
                sc[b][u] = _dot_nt(qabs[b * H:(b + 1) * H],
                                   ckv_v[b, u * UR:(u + 1) * UR, :]) * scale

        def b_softmax(b):
            s = jnp.concatenate(sc[b], axis=1)
            m = jnp.max(s, axis=-1, keepdims=True)
            p = jnp.exp(s - m)
            l = jnp.sum(p, axis=-1, keepdims=True)
            return p.astype(_BF16), l

        def b_ctx(b, p, l):
            cc = _dot(p, ckv_v[b])
            return (cc / l).astype(_BF16)

        issue_ckv(4)
        b_scores(0)
        b_scores(1)
        issue_ckv(5)
        b_scores(2)
        issue_ckv(6)
        b_scores(3)
        issue_ckv(7)
        b_scores(4)
        issue_w3(2, wuv_hbm, wuv_v, 0)
        b_scores(5)
        issue_w3(2, wuv_hbm, wuv_v, 1)
        b_scores(6)
        issue_w512(wob_hbm, wob_v, sem.at[3], 0)
        b_scores(7)
        p0, l0 = b_softmax(0)
        issue_w512(wob_hbm, wob_v, sem.at[3], 1)
        p1, l1 = b_softmax(1)
        cc0 = b_ctx(0, p0, l0)
        issue_wq(0)
        cc1 = b_ctx(1, p1, l1)
        ctxc = jnp.concatenate([cc0, cc1], axis=0)
        issue_wq(1)
        ctx = project_j(ctxc, 2, wuv_v, 0) + project_j(ctxc, 2, wuv_v, 2)
        issue_w512(wo_hbm, wo_v, sem.at[4], 0)
        issue_w512(wo_hbm, wo_v, sem.at[4], 1)
        ctx = ctx + project_j(ctxc, 2, wuv_v, 1) + project_j(ctxc, 2, wuv_v, 3)
        for part in range(NP // 2):
            issue_chunk_part(0, part)

        _wait_full(wob_v, sem.at[3])
        dmask = (jax.lax.broadcasted_iota(jnp.int32, (R, H * Dh), 1) // Dh
                 == jax.lax.broadcasted_iota(jnp.int32, (R, H * Dh), 0) % H)
        l2 = jnp.where(dmask, jnp.tile(ctx, (1, H)), 0.0).astype(_BF16)
        yb = _dot(l2, wob_v[...])
        outb = [jnp.sum(yb[b * H:(b + 1) * H], axis=0, keepdims=True) for b in range(B)]

        gw = gw_v[...].astype(_F32).reshape(1, D)
        gate = jax.nn.sigmoid(jnp.sum(xav * gw, axis=-1, keepdims=True))
        base = (1.0 - gate) * jnp.concatenate(outb, axis=0)

        _wait_full(wq_v, sem.at[2])
        xa = jnp.concatenate(
            [jnp.broadcast_to(xav[b:b + 1], (8, D)) for b in range(B)], axis=0).astype(_BF16)
        qa = _dot(xa, wq_v[...])
        for b in range(B):
            for h in range(H):
                q_s[b * H + h] = qa[b * 8:(b + 1) * 8, h * Dh:(h + 1) * Dh].astype(_BF16)
        acc_s[...] = jnp.zeros_like(acc_s)
        for part in range(NP // 2, NP):
            issue_chunk_part(0, part)
        _wait_full(wo_v, sem.at[4])

        NMAIN = BH - HPC

        def softmax_probs(i, kval):
            sc_ = _dot_nt(q_s[i], kval) * scale
            m = jnp.max(sc_, axis=-1, keepdims=True)
            p = jnp.exp(sc_ - m)
            l = jnp.sum(p, axis=-1, keepdims=True)
            return p.astype(_BF16), l

        def issue_for(i, u):
            c = i // HPC
            hh = i % HPC

            @pl.when(i < NMAIN - HPC)
            def _():
                issue_chunk_part(c + 1, hh * NPART + u)

            if u == 0:
                e = i - (NMAIN - HPC)

                @pl.when(jnp.logical_and(e >= 0, e < 2 * (HPC - 1)))
                def _():
                    issue_last_part(e // 2, e % 2)

                @pl.when(e == 2 * (HPC - 1))
                def _():
                    issue_last_head()

        def step(i, carry):
            c = i // HPC
            hh = i % HPC
            slot = c % NSLOT
            blk = pl.ds(2 * hh, 2)

            issue_for(i, 0)

            @pl.when(jnp.logical_and(i < NMAIN, hh == 0))
            def _():
                _wait_full(kbuf.at[slot], ksem.at[slot])

            @pl.when(i >= NMAIN)
            def _():
                _wait_full(kbuf.at[LSLOT, blk], hsem.at[0, hh])

            p, l = softmax_probs(i, kbuf[slot, blk].reshape(Sk, Dh))

            issue_for(i, 1)

            @pl.when(jnp.logical_and(i < NMAIN, hh == 0))
            def _():
                _wait_full(vbuf.at[slot], vsem.at[slot])

            @pl.when(i >= NMAIN)
            def _():
                _wait_full(vbuf.at[LSLOT, blk], hsem.at[1, hh])

            o = _dot(p, vbuf[slot, blk].reshape(Sk, Dh)) / l
            h = i % H
            y = _dot(o.astype(_BF16), wo_v[pl.ds(pl.multiple_of(h * Dh, Dh), Dh), :])
            acc_s[i // H] = acc_s[i // H] + y
            return carry

        jax.lax.fori_loop(0, BH - 1, step, 0)

        i = BH - 1
        b0 = 2 * (HPC - 1)
        _wait_full(kbuf.at[LSLOT, pl.ds(b0, 2)], hsem.at[0, HPC - 1])
        p, l = softmax_probs(i, kbuf[LSLOT, b0:b0 + 2].reshape(Sk, Dh))
        o = jnp.zeros((8, Dh), _F32)
        for pc in range(VPIECES):
            r0 = pc * PR
            _wait_full(vbuf.at[LSLOT, pl.ds(b0, 2), pl.ds(r0, PR)], lsem.at[pc])
            pp = jnp.concatenate([p[:, r0:r0 + PR], p[:, HS + r0:HS + r0 + PR]], axis=1)
            o = o + _dot(pp, vbuf[LSLOT, b0:b0 + 2, r0:r0 + PR, :].reshape(2 * PR, Dh))
        o = o / l
        y = _dot(o.astype(_BF16), wo_v[(H - 1) * Dh:H * Dh, :])
        a = jnp.concatenate([acc_s[0][0:1], acc_s[1][0:1] + y[0:1]], axis=0)
        out_v[...] = (gate * a + base).astype(out_v.dtype)
        c_out = pltpu.make_async_copy(out_v, out_hbm, osem.at[0])
        c_out.start()
        c_out.wait()

    any_spec = pl.BlockSpec(memory_space=pl.ANY)
    bf = _BF16
    out = pl.pallas_call(
        kernel,
        in_specs=[any_spec] * 11,
        out_specs=any_spec,
        out_shape=jax.ShapeDtypeStruct((B, D), A_x.dtype),
        scratch_shapes=[
            pltpu.VMEM((B, D), bf),
            pltpu.VMEM((D,), bf),
            pltpu.VMEM((D, H * Dh), bf),
            pltpu.VMEM((H * Dh, D), bf),
            pltpu.VMEM((B, Sk, Dc), bf),
            pltpu.VMEM((M * H, Dh), bf),
            pltpu.VMEM((Dc * H, Dh), bf),
            pltpu.VMEM((Dc * H, Dh), bf),
            pltpu.VMEM((H * Dh, M), bf),
            pltpu.VMEM((NSLOT, NBLK, HS, Dh), bf),
            pltpu.VMEM((NSLOT, NBLK, HS, Dh), bf),
            pltpu.VMEM((BH, 8, Dh), bf),
            pltpu.VMEM((B, 8, D), _F32),
            pltpu.VMEM((B, D), bf),
            pltpu.SemaphoreType.DMA((5,)),
            pltpu.SemaphoreType.DMA((3, NJ)),
            pltpu.SemaphoreType.DMA((B, NU)),
            pltpu.SemaphoreType.DMA((NSLOT,)),
            pltpu.SemaphoreType.DMA((NSLOT,)),
            pltpu.SemaphoreType.DMA((2, HPC)),
            pltpu.SemaphoreType.DMA((VPIECES,)),
            pltpu.SemaphoreType.DMA((1,)),
        ],
        compiler_params=pltpu.CompilerParams(vmem_limit_bytes=110 * 1024 * 1024,
                                             disable_semaphore_checks=True),
    )(xa2, gate_w, k3, v3, A_wq, A_wo, B_c_kv, wqb2, wuk2, wuv2, wob2)
    return out.reshape(B, Sq, D)
```

```python
import jax
import jax.numpy as jnp
import jax.experimental.pallas as pl
import jax.experimental.pallas.tpu as pltpu

_NT = (((1,), (1,)), ((), ()))
_F32 = jnp.float32
_BF16 = jnp.bfloat16

NSLOT = 2
HPC = 4
NBLK = 2 * HPC
KVSUB = 16
LSUB = 96
NPART = 2
VPIECES = 4


def _dot(a, b):
    return jnp.dot(a, b, preferred_element_type=_F32)


def _dot_nt(a, b):
    return jax.lax.dot_general(a, b, _NT, preferred_element_type=_F32)


def _wait_full(buf, sem):
    pltpu.make_async_copy(buf, buf, sem).wait()


@jax.jit
def pallas_gated_mix__mha_block_cached__compressed_kv_cla__decode_kernel(
    A_x: jax.Array,
    A_k_cache: jax.Array,
    A_v_cache: jax.Array,
    A_wq: jax.Array,
    A_wo: jax.Array,
    B_x: jax.Array,
    B_c_kv: jax.Array,
    B_w_q: jax.Array,
    B_w_uk: jax.Array,
    B_w_uv: jax.Array,
    B_w_o: jax.Array,
    gate_w: jax.Array,
):
    B, Sq, D = A_x.shape
    _, H, Sk, Dh = A_k_cache.shape
    Dc = B_c_kv.shape[-1]
    M = B_w_q.shape[0]
    assert Sq == 1 and B == 2 and Dh == 128 and H == 32 and D == 512 and M == D and Dc == 512
    BH = B * H
    R = BH
    NJ = Dc // 128
    CH = 128 * H
    scale = float(Dh) ** -0.5
    NU = 8
    UR = Sk // NU
    UB = UR // NU
    PR = (Sk // 2) // VPIECES

    xa2 = A_x.reshape(B, D)
    HS = Sk // 2
    NCH = BH // HPC
    k3 = A_k_cache.reshape(NCH, NBLK, HS, Dh)
    v3 = A_v_cache.reshape(NCH, NBLK, HS, Dh)
    wqb2 = B_w_q.reshape(NJ, CH, Dh)
    wuk2 = B_w_uk.reshape(NJ, CH, Dh)
    wuv2 = B_w_uv.reshape(NJ, CH, Dh)
    wob2 = B_w_o.reshape(4, H * Dh // 4, M)
    wo2 = A_wo.reshape(4, H * Dh // 4, D)
    wq2 = A_wq.reshape(4, D // 4, H * Dh)
    ckv4 = B_c_kv.reshape(B, NU, UR, Dc)

    def kernel(xa_hbm, gw_hbm, k_hbm, v_hbm, wq_hbm, wo_hbm, ckv_hbm,
               wqb_hbm, wuk_hbm, wuv_hbm, wob_hbm,
               out_hbm,
               xa_v, gw_v, wq_v, wo_v, ckv_v, wqb_v, wuk_v, wuv_v, wob_v,
               kbuf, vbuf, q_s, acc_s, out_v,
               sem, csem, ksem, vsem, hsem, lsem, osem):

        def d_w3(src, dst, sm, t):
            r = pl.ds(pl.multiple_of(t * 32, 32), 32)
            return pltpu.make_async_copy(src.at[:, r], dst.at[:, r], sm)

        def d_w512(src, dst, sm, t):
            r = pl.ds(pl.multiple_of(t * 8, 8), 8)
            return pltpu.make_async_copy(src.at[:, r], dst.at[:, r], sm)

        def d_wq(src, dst, sm, t):
            r = pl.ds(pl.multiple_of((t // 8) * 8, 8), 8)
            c = pl.ds(pl.multiple_of((t % 8) * 512, 512), 512)
            return pltpu.make_async_copy(src.at[:, r, c], dst.at[:, r, c], sm)

        def d_ckv(src, dst, sm, t):
            r = pl.ds(pl.multiple_of((t // 2) * 8, 8), 8)
            c = pl.ds(pl.multiple_of((t % 2) * 256, 256), 256)
            return pltpu.make_async_copy(src.at[:, r, c], dst.at[:, r, c], sm)

        def issue_unit(d0, a0, d1, a1, u, n=32):
            def one(t, c):
                d0(*a0, t).start(priority=0)
                d1(*a1, t).start(priority=1)
                return c

            jax.lax.fori_loop(u * n, (u + 1) * n, one, 0, unroll=4)

        def issue_s1(u):
            issue_unit(d_w3, (wqb_hbm, wqb_v, sem.at[5]), d_w3, (wuk_hbm, wuk_v, sem.at[6]), u)

        def issue_ckv(u):
            issue_unit(d_ckv, (ckv_hbm.at[0], ckv_v.at[0], csem.at[0, u]),
                       d_ckv, (ckv_hbm.at[1], ckv_v.at[1], csem.at[1, u]), u, n=UB // 4)

        def issue_s3(u):
            issue_unit(d_w3, (wuv_hbm, wuv_v, sem.at[7]), d_w512, (wob_hbm, wob_v, sem.at[3]), u)

        def issue_s4(u):
            issue_unit(d_wq, (wq_hbm, wq_v, sem.at[2]), d_w512, (wo_hbm, wo_v, sem.at[4]), u)

        def kv_pairs(ksrc, kdst, ks, vsrc, vdst, vs, r0, rows, sub):
            nfull = rows // sub
            rem = rows - nfull * sub

            def pair(off, n):
                pltpu.make_async_copy(ksrc.at[:, pl.ds(off, n)], kdst.at[:, pl.ds(off, n)], ks).start(priority=0)
                pltpu.make_async_copy(vsrc.at[:, pl.ds(off, n)], vdst.at[:, pl.ds(off, n)], vs).start(priority=1)

            def one(t, c):
                pair(pl.multiple_of(r0 + t * sub, 16), sub)
                return c

            jax.lax.fori_loop(0, nfull, one, 0, unroll=4)
            if rem:
                pair(r0 + nfull * sub, rem)

        NP = HPC * NPART
        PROWS = HS // NP

        def issue_chunk_part(c, part):
            slot = c % NSLOT
            kv_pairs(k_hbm.at[c], kbuf.at[slot], ksem.at[slot], v_hbm.at[c], vbuf.at[slot], vsem.at[slot],
                     part * PROWS, PROWS, KVSUB)

        LSLOT = (NCH - 1) % NSLOT

        def issue_last_part(hh, u):
            blk = pl.ds(2 * hh, 2)
            kv_pairs(k_hbm.at[NCH - 1, blk], kbuf.at[LSLOT, blk], hsem.at[0, hh],
                     v_hbm.at[NCH - 1, blk], vbuf.at[LSLOT, blk], hsem.at[1, hh],
                     u * (HS // NPART), HS // NPART, LSUB)

        def issue_last_head():
            hh = HPC - 1
            blk = pl.ds(2 * hh, 2)
            for p in range(VPIECES):
                kv_pairs(k_hbm.at[NCH - 1, blk], kbuf.at[LSLOT, blk], hsem.at[0, hh],
                         v_hbm.at[NCH - 1, blk], vbuf.at[LSLOT, blk], lsem.at[p], p * PR, PR, LSUB)

        c_xa = pltpu.make_async_copy(xa_hbm, xa_v, sem.at[0])
        c_gw = pltpu.make_async_copy(gw_hbm, gw_v, sem.at[1])
        issue_s1(0)
        c_xa.start()
        c_gw.start()
        issue_s1(1)

        st = (jax.lax.broadcasted_iota(jnp.int32, (128, CH), 1) // H
              == jax.lax.broadcasted_iota(jnp.int32, (128, CH), 0)).astype(_F32).astype(_BF16)
        issue_s1(2)
        s_ = (jax.lax.broadcasted_iota(jnp.int32, (CH, 128), 0) // H
              == jax.lax.broadcasted_iota(jnp.int32, (CH, 128), 1)).astype(_F32).astype(_BF16)
        hmask = (jax.lax.broadcasted_iota(jnp.int32, (R, CH), 1) % H
                 == jax.lax.broadcasted_iota(jnp.int32, (R, CH), 0) % H)

        def project_j(c, w_ref, j):
            e = _dot(c[:, j * 128:(j + 1) * 128], st)
            l = jnp.where(hmask, e, 0.0).astype(_BF16)
            return _dot(l, w_ref[j])

        issue_s1(3)
        issue_ckv(0)
        issue_ckv(1)
        c_xa.wait()
        c_gw.wait()
        xav = xa_v[...].astype(_F32)
        xb = jnp.concatenate(
            [jnp.broadcast_to(xav[b:b + 1], (H, M)) for b in range(B)], axis=0).astype(_BF16)
        _wait_full(wqb_v, sem.at[5])
        qb = project_j(xb, wqb_v, 0) + project_j(xb, wqb_v, 1)
        issue_ckv(2)
        qb = qb + project_j(xb, wqb_v, 2) + project_j(xb, wqb_v, 3)
        qb = qb.astype(_BF16)

        def absorb_j(j):
            t = _dot_nt(qb, wuk_v[j])
            t = jnp.where(hmask, t, 0.0).astype(_BF16)
            return _dot(t, s_).astype(_BF16)

        issue_ckv(3)
        _wait_full(wuk_v, sem.at[6])
        qabs = [absorb_j(0), absorb_j(1)]
        issue_ckv(4)
        qabs += [absorb_j(2), absorb_j(3)]
        qabs = jnp.concatenate(qabs, axis=1)

        sc = [[None] * NU for _ in range(B)]

        def ckv_unit(b, u):
            return ckv_v[b, :, u * UB:(u + 1) * UB, :].reshape(NU * UB, Dc)

        def b_scores(u):
            for b in range(B):
                _wait_full(ckv_v.at[b, :, pl.ds(u * UB, UB)], csem.at[b, u])
                sc[b][u] = _dot_nt(qabs[b * H:(b + 1) * H], ckv_unit(b, u)) * scale

        def b_softmax(b):
            s = jnp.concatenate(sc[b], axis=1)
            m = jnp.max(s, axis=-1, keepdims=True)
            p = jnp.exp(s - m)
            l = jnp.sum(p, axis=-1, keepdims=True)
            return p.astype(_BF16), l

        def b_ctx(b, p, l):
            cc = _dot(p[:, 0:NU * UB], ckv_unit(b, 0))
            for u in range(1, NU):
                cc = cc + _dot(p[:, u * NU * UB:(u + 1) * NU * UB], ckv_unit(b, u))
            return (cc / l).astype(_BF16)

        issue_ckv(5)
        b_scores(0)
        b_scores(1)
        issue_ckv(6)
        b_scores(2)
        b_scores(3)
        issue_ckv(7)
        b_scores(4)
        b_scores(5)
        issue_s3(0)
        b_scores(6)
        issue_s3(1)
        b_scores(7)
        p0, l0 = b_softmax(0)
        issue_s3(2)
        p1, l1 = b_softmax(1)
        issue_s3(3)
        cc0 = b_ctx(0, p0, l0)
        issue_s4(0)
        cc1 = b_ctx(1, p1, l1)
        ctxc = jnp.concatenate([cc0, cc1], axis=0)
        issue_s4(1)
        _wait_full(wuv_v, sem.at[7])
        ctx = project_j(ctxc, wuv_v, 0) + project_j(ctxc, wuv_v, 1)
        issue_s4(2)
        ctx = ctx + project_j(ctxc, wuv_v, 2) + project_j(ctxc, wuv_v, 3)
        issue_s4(3)

        _wait_full(wob_v, sem.at[3])
        dmask = (jax.lax.broadcasted_iota(jnp.int32, (R, H * Dh), 1) // Dh
                 == jax.lax.broadcasted_iota(jnp.int32, (R, H * Dh), 0) % H)
        l2 = jnp.where(dmask, jnp.tile(ctx, (1, H)), 0.0).astype(_BF16)
        yb = _dot(l2, wob_v[...].reshape(H * Dh, M))
        outb = [jnp.sum(yb[b * H:(b + 1) * H], axis=0, keepdims=True) for b in range(B)]
        issue_chunk_part(0, 0)

        gw = gw_v[...].astype(_F32).reshape(1, D)
        gate = jax.nn.sigmoid(jnp.sum(xav * gw, axis=-1, keepdims=True))
        base = (1.0 - gate) * jnp.concatenate(outb, axis=0)
        issue_chunk_part(0, 1)

        _wait_full(wq_v, sem.at[2])
        xa = jnp.concatenate(
            [jnp.broadcast_to(xav[b:b + 1], (8, D)) for b in range(B)], axis=0).astype(_BF16)
        qa = _dot(xa, wq_v[...].reshape(D, H * Dh))
        for b in range(B):
            for h in range(H):
                q_s[b * H + h] = qa[b * 8:(b + 1) * 8, h * Dh:(h + 1) * Dh].astype(_BF16)
        acc_s[...] = jnp.zeros_like(acc_s)
        for part in range(2, NP):
            issue_chunk_part(0, part)
        _wait_full(wo_v, sem.at[4])

        NMAIN = BH - HPC

        def softmax_probs(i, kval):
            sc_ = _dot_nt(q_s[i], kval) * scale
            m = jnp.max(sc_, axis=-1, keepdims=True)
            p = jnp.exp(sc_ - m)
            l = jnp.sum(p, axis=-1, keepdims=True)
            return p.astype(_BF16), l

        def issue_for(i, u):
            c = i // HPC
            hh = i % HPC

            @pl.when(i < NMAIN - HPC)
            def _():
                issue_chunk_part(c + 1, hh * NPART + u)

            if u == 0:
                e = i - (NMAIN - HPC)

                @pl.when(jnp.logical_and(e >= 0, e < 2 * (HPC - 1)))
                def _():
                    issue_last_part(e // 2, e % 2)

                @pl.when(e == 2 * (HPC - 1))
                def _():
                    issue_last_head()

        def step(i, carry):
            c = i // HPC
            hh = i % HPC
            slot = c % NSLOT
            blk = pl.ds(2 * hh, 2)

            issue_for(i, 0)

            @pl.when(jnp.logical_and(i < NMAIN, hh == 0))
            def _():
                _wait_full(kbuf.at[slot], ksem.at[slot])

            @pl.when(i >= NMAIN)
            def _():
                _wait_full(kbuf.at[LSLOT, blk], hsem.at[0, hh])

            p, l = softmax_probs(i, kbuf[slot, blk].reshape(Sk, Dh))

            issue_for(i, 1)

            @pl.when(jnp.logical_and(i < NMAIN, hh == 0))
            def _():
                _wait_full(vbuf.at[slot], vsem.at[slot])

            @pl.when(i >= NMAIN)
            def _():
                _wait_full(vbuf.at[LSLOT, blk], hsem.at[1, hh])

            o = _dot(p, vbuf[slot, blk].reshape(Sk, Dh)) / l
            h = i % H
            y = _dot(o.astype(_BF16), wo_v[h // 8, pl.ds(pl.multiple_of((h % 8) * Dh, Dh), Dh), :])
            acc_s[i // H] = acc_s[i // H] + y
            return carry

        jax.lax.fori_loop(0, BH - 1, step, 0)

        i = BH - 1
        b0 = 2 * (HPC - 1)
        _wait_full(kbuf.at[LSLOT, pl.ds(b0, 2)], hsem.at[0, HPC - 1])
        p, l = softmax_probs(i, kbuf[LSLOT, b0:b0 + 2].reshape(Sk, Dh))
        o = jnp.zeros((8, Dh), _F32)
        for pc in range(VPIECES):
            r0 = pc * PR
            _wait_full(vbuf.at[LSLOT, pl.ds(b0, 2), pl.ds(r0, PR)], lsem.at[pc])
            pp = jnp.concatenate([p[:, r0:r0 + PR], p[:, HS + r0:HS + r0 + PR]], axis=1)
            o = o + _dot(pp, vbuf[LSLOT, b0:b0 + 2, r0:r0 + PR, :].reshape(2 * PR, Dh))
        o = o / l
        y = _dot(o.astype(_BF16), wo_v[3, 7 * Dh:8 * Dh, :])
        a = jnp.concatenate([acc_s[0][0:1], acc_s[1][0:1] + y[0:1]], axis=0)
        out_v[...] = (gate * a + base).astype(out_v.dtype)
        c_out = pltpu.make_async_copy(out_v, out_hbm, osem.at[0])
        c_out.start()
        c_out.wait()

    any_spec = pl.BlockSpec(memory_space=pl.ANY)
    bf = _BF16
    out = pl.pallas_call(
        kernel,
        in_specs=[any_spec] * 11,
        out_specs=any_spec,
        out_shape=jax.ShapeDtypeStruct((B, D), A_x.dtype),
        scratch_shapes=[
            pltpu.VMEM((B, D), bf),
            pltpu.VMEM((D,), bf),
            pltpu.VMEM((4, D // 4, H * Dh), bf),
            pltpu.VMEM((4, H * Dh // 4, D), bf),
            pltpu.VMEM((B, NU, UR, Dc), bf),
            pltpu.VMEM((NJ, CH, Dh), bf),
            pltpu.VMEM((NJ, CH, Dh), bf),
            pltpu.VMEM((NJ, CH, Dh), bf),
            pltpu.VMEM((4, H * Dh // 4, M), bf),
            pltpu.VMEM((NSLOT, NBLK, HS, Dh), bf),
            pltpu.VMEM((NSLOT, NBLK, HS, Dh), bf),
            pltpu.VMEM((BH, 8, Dh), bf),
            pltpu.VMEM((B, 8, D), _F32),
            pltpu.VMEM((B, D), bf),
            pltpu.SemaphoreType.DMA((8,)),
            pltpu.SemaphoreType.DMA((B, NU)),
            pltpu.SemaphoreType.DMA((NSLOT,)),
            pltpu.SemaphoreType.DMA((NSLOT,)),
            pltpu.SemaphoreType.DMA((2, HPC)),
            pltpu.SemaphoreType.DMA((VPIECES,)),
            pltpu.SemaphoreType.DMA((1,)),
        ],
        compiler_params=pltpu.CompilerParams(vmem_limit_bytes=110 * 1024 * 1024,
                                             disable_semaphore_checks=True),
    )(xa2, gate_w, k3, v3, wq2, wo2, ckv4, wqb2, wuk2, wuv2, wob2)
    return out.reshape(B, Sq, D)
```

```python
import jax
import jax.numpy as jnp
import jax.experimental.pallas as pl
import jax.experimental.pallas.tpu as pltpu

_NT = (((1,), (1,)), ((), ()))
_F32 = jnp.float32
_BF16 = jnp.bfloat16

NSLOT = 2
HPC = 5
LH = 4
NBLK = 2 * HPC
KVSUB = 16
LSUB = 96
NPART = 2
NP = 8
VPIECES = 4


def _dot(a, b):
    return jnp.dot(a, b, preferred_element_type=_F32)


def _dot_nt(a, b):
    return jax.lax.dot_general(a, b, _NT, preferred_element_type=_F32)


def _wait_full(buf, sem):
    pltpu.make_async_copy(buf, buf, sem).wait()


@jax.jit
def pallas_gated_mix__mha_block_cached__compressed_kv_cla__decode_kernel(
    A_x: jax.Array,
    A_k_cache: jax.Array,
    A_v_cache: jax.Array,
    A_wq: jax.Array,
    A_wo: jax.Array,
    B_x: jax.Array,
    B_c_kv: jax.Array,
    B_w_q: jax.Array,
    B_w_uk: jax.Array,
    B_w_uv: jax.Array,
    B_w_o: jax.Array,
    gate_w: jax.Array,
):
    B, Sq, D = A_x.shape
    _, H, Sk, Dh = A_k_cache.shape
    Dc = B_c_kv.shape[-1]
    M = B_w_q.shape[0]
    assert Sq == 1 and B == 2 and Dh == 128 and H == 32 and D == 512 and M == D and Dc == 512
    BH = B * H
    R = BH
    NJ = Dc // 128
    CH = 128 * H
    scale = float(Dh) ** -0.5
    NU = 8
    UR = Sk // NU
    UB = UR // NU
    PR = (Sk // 2) // VPIECES

    xa2 = A_x.reshape(B, D)
    HS = Sk // 2
    NMAIN = BH - LH
    NCH = NMAIN // HPC
    assert NCH * HPC == NMAIN and NP <= NPART * HPC
    k3 = A_k_cache.reshape(2 * BH, HS, Dh)
    v3 = A_v_cache.reshape(2 * BH, HS, Dh)
    wqb2 = B_w_q.reshape(NJ, CH, Dh)
    wuk2 = B_w_uk.reshape(NJ, CH, Dh)
    wuv2 = B_w_uv.reshape(NJ, CH, Dh)
    wob2 = B_w_o.reshape(4, H * Dh // 4, M)
    wo2 = A_wo.reshape(4, H * Dh // 4, D)
    wq2 = A_wq.reshape(4, D // 4, H * Dh)
    ckv4 = B_c_kv.reshape(B, NU, UR, Dc)

    def kernel(xa_hbm, gw_hbm, k_hbm, v_hbm, wq_hbm, wo_hbm, ckv_hbm,
               wqb_hbm, wuk_hbm, wuv_hbm, wob_hbm,
               out_hbm,
               xa_v, gw_v, wq_v, wo_v, ckv_v, wqb_v, wuk_v, wuv_v, wob_v,
               kbuf, vbuf, q_s, acc_s, out_v,
               sem, csem, ksem, vsem, hsem, lsem, osem):

        def d_w3(src, dst, sm, t):
            r = pl.ds(pl.multiple_of(t * 32, 32), 32)
            return pltpu.make_async_copy(src.at[:, r], dst.at[:, r], sm)

        def d_w512(src, dst, sm, t):
            r = pl.ds(pl.multiple_of(t * 8, 8), 8)
            return pltpu.make_async_copy(src.at[:, r], dst.at[:, r], sm)

        def d_wq(src, dst, sm, t):
            r = pl.ds(pl.multiple_of((t // 8) * 8, 8), 8)
            c = pl.ds(pl.multiple_of((t % 8) * 512, 512), 512)
            return pltpu.make_async_copy(src.at[:, r, c], dst.at[:, r, c], sm)

        def d_ckv(src, dst, sm, t):
            r = pl.ds(pl.multiple_of((t // 2) * 8, 8), 8)
            c = pl.ds(pl.multiple_of((t % 2) * 256, 256), 256)
            return pltpu.make_async_copy(src.at[:, r, c], dst.at[:, r, c], sm)

        def issue_unit(d0, a0, d1, a1, u, n=32):
            def one(t, c):
                d1(*a1, t).start(priority=1)
                d0(*a0, t).start(priority=0)
                return c

            jax.lax.fori_loop(u * n, (u + 1) * n, one, 0, unroll=4)

        def issue_s1(u):
            issue_unit(d_w3, (wqb_hbm, wqb_v, sem.at[5]), d_w3, (wuk_hbm, wuk_v, sem.at[6]), u)

        def issue_ckv(u):
            issue_unit(d_ckv, (ckv_hbm.at[0], ckv_v.at[0], csem.at[0, u]),
                       d_ckv, (ckv_hbm.at[1], ckv_v.at[1], csem.at[1, u]), u, n=UB // 4)

        def issue_s3(u):
            issue_unit(d_w3, (wuv_hbm, wuv_v, sem.at[7]), d_w512, (wob_hbm, wob_v, sem.at[3]), u)

        def issue_s4(u):
            issue_unit(d_wq, (wq_hbm, wq_v, sem.at[2]), d_w512, (wo_hbm, wo_v, sem.at[4]), u)

        def kv_pairs(ksrc, kdst, ks, vsrc, vdst, vs, r0, rows, sub):
            nfull = rows // sub
            rem = rows - nfull * sub

            def pair(off, n):
                pltpu.make_async_copy(vsrc.at[:, pl.ds(off, n)], vdst.at[:, pl.ds(off, n)], vs).start(priority=1)
                pltpu.make_async_copy(ksrc.at[:, pl.ds(off, n)], kdst.at[:, pl.ds(off, n)], ks).start(priority=0)

            def one(t, c):
                pair(pl.multiple_of(r0 + t * sub, 16), sub)
                return c

            jax.lax.fori_loop(0, nfull, one, 0, unroll=4)
            if rem:
                pair(r0 + nfull * sub, rem)

        PROWS = HS // NP

        def issue_chunk_part(c, part):
            slot = c % NSLOT
            blk = pl.ds(c * NBLK, NBLK)
            kv_pairs(k_hbm.at[blk], kbuf.at[slot], ksem.at[slot], v_hbm.at[blk], vbuf.at[slot], vsem.at[slot],
                     part * PROWS, PROWS, KVSUB)

        LSLOT = NCH % NSLOT

        def issue_last_part(hh, u):
            src = pl.ds(2 * (NMAIN + hh), 2)
            dst = pl.ds(2 * hh, 2)
            kv_pairs(k_hbm.at[src], kbuf.at[LSLOT, dst], hsem.at[0, hh],
                     v_hbm.at[src], vbuf.at[LSLOT, dst], hsem.at[1, hh],
                     u * (HS // NPART), HS // NPART, LSUB)

        def issue_last_head():
            hh = LH - 1
            src = pl.ds(2 * (NMAIN + hh), 2)
            dst = pl.ds(2 * hh, 2)
            for p in range(VPIECES):
                kv_pairs(k_hbm.at[src], kbuf.at[LSLOT, dst], hsem.at[0, hh],
                         v_hbm.at[src], vbuf.at[LSLOT, dst], lsem.at[p], p * PR, PR, LSUB)

        c_xa = pltpu.make_async_copy(xa_hbm, xa_v, sem.at[0])
        c_gw = pltpu.make_async_copy(gw_hbm, gw_v, sem.at[1])
        issue_s1(0)
        c_xa.start()
        c_gw.start()
        issue_s1(1)

        st = (jax.lax.broadcasted_iota(jnp.int32, (128, CH), 1) // H
              == jax.lax.broadcasted_iota(jnp.int32, (128, CH), 0)).astype(_F32).astype(_BF16)
        issue_s1(2)
        s_ = (jax.lax.broadcasted_iota(jnp.int32, (CH, 128), 0) // H
              == jax.lax.broadcasted_iota(jnp.int32, (CH, 128), 1)).astype(_F32).astype(_BF16)
        hmask = (jax.lax.broadcasted_iota(jnp.int32, (R, CH), 1) % H
                 == jax.lax.broadcasted_iota(jnp.int32, (R, CH), 0) % H)

        def project_j(c, w_ref, j):
            e = _dot(c[:, j * 128:(j + 1) * 128], st)
            l = jnp.where(hmask, e, 0.0).astype(_BF16)
            return _dot(l, w_ref[j])

        issue_s1(3)
        issue_ckv(0)
        issue_ckv(1)
        c_xa.wait()
        c_gw.wait()
        xav = xa_v[...].astype(_F32)
        xb = jnp.concatenate(
            [jnp.broadcast_to(xav[b:b + 1], (H, M)) for b in range(B)], axis=0).astype(_BF16)
        _wait_full(wqb_v, sem.at[5])
        qb = project_j(xb, wqb_v, 0) + project_j(xb, wqb_v, 1)
        issue_ckv(2)
        qb = qb + project_j(xb, wqb_v, 2) + project_j(xb, wqb_v, 3)
        qb = qb.astype(_BF16)

        def absorb_j(j):
            t = _dot_nt(qb, wuk_v[j])
            t = jnp.where(hmask, t, 0.0).astype(_BF16)
            return _dot(t, s_).astype(_BF16)

        issue_ckv(3)
        _wait_full(wuk_v, sem.at[6])
        qabs = [absorb_j(0), absorb_j(1)]
        issue_ckv(4)
        qabs += [absorb_j(2), absorb_j(3)]
        qabs = jnp.concatenate(qabs, axis=1)

        sc = [[None] * NU for _ in range(B)]

        def ckv_unit(b, u):
            return ckv_v[b, :, u * UB:(u + 1) * UB, :].reshape(NU * UB, Dc)

        def b_scores(u):
            for b in range(B):
                _wait_full(ckv_v.at[b, :, pl.ds(u * UB, UB)], csem.at[b, u])
                sc[b][u] = _dot_nt(qabs[b * H:(b + 1) * H], ckv_unit(b, u)) * scale

        def b_softmax(b):
            s = jnp.concatenate(sc[b], axis=1)
            m = jnp.max(s, axis=-1, keepdims=True)
            p = jnp.exp(s - m)
            l = jnp.sum(p, axis=-1, keepdims=True)
            return p.astype(_BF16), l

        def b_ctx(b, p, l):
            cc = _dot(p[:, 0:NU * UB], ckv_unit(b, 0))
            for u in range(1, NU):
                cc = cc + _dot(p[:, u * NU * UB:(u + 1) * NU * UB], ckv_unit(b, u))
            return (cc / l).astype(_BF16)

        issue_ckv(5)
        b_scores(0)
        b_scores(1)
        issue_ckv(6)
        b_scores(2)
        b_scores(3)
        issue_ckv(7)
        b_scores(4)
        b_scores(5)
        issue_s3(0)
        b_scores(6)
        issue_s3(1)
        b_scores(7)
        p0, l0 = b_softmax(0)
        issue_s3(2)
        p1, l1 = b_softmax(1)
        issue_s3(3)
        cc0 = b_ctx(0, p0, l0)
        issue_s4(0)
        cc1 = b_ctx(1, p1, l1)
        ctxc = jnp.concatenate([cc0, cc1], axis=0)
        issue_s4(1)
        _wait_full(wuv_v, sem.at[7])
        ctx = project_j(ctxc, wuv_v, 0) + project_j(ctxc, wuv_v, 1)
        issue_s4(2)
        ctx = ctx + project_j(ctxc, wuv_v, 2) + project_j(ctxc, wuv_v, 3)
        issue_s4(3)

        _wait_full(wob_v, sem.at[3])
        dmask = (jax.lax.broadcasted_iota(jnp.int32, (R, H * Dh), 1) // Dh
                 == jax.lax.broadcasted_iota(jnp.int32, (R, H * Dh), 0) % H)
        l2 = jnp.where(dmask, jnp.tile(ctx, (1, H)), 0.0).astype(_BF16)
        yb = _dot(l2, wob_v[...].reshape(H * Dh, M))
        outb = [jnp.sum(yb[b * H:(b + 1) * H], axis=0, keepdims=True) for b in range(B)]
        issue_chunk_part(0, 0)

        gw = gw_v[...].astype(_F32).reshape(1, D)
        gate = jax.nn.sigmoid(jnp.sum(xav * gw, axis=-1, keepdims=True))
        base = (1.0 - gate) * jnp.concatenate(outb, axis=0)
        issue_chunk_part(0, 1)

        _wait_full(wq_v, sem.at[2])
        xa = jnp.concatenate(
            [jnp.broadcast_to(xav[b:b + 1], (8, D)) for b in range(B)], axis=0).astype(_BF16)
        qa = _dot(xa, wq_v[...].reshape(D, H * Dh))
        for b in range(B):
            for h in range(H):
                q_s[b * H + h] = qa[b * 8:(b + 1) * 8, h * Dh:(h + 1) * Dh].astype(_BF16)
        acc_s[...] = jnp.zeros_like(acc_s)
        for part in range(2, NP):
            issue_chunk_part(0, part)
        _wait_full(wo_v, sem.at[4])

        def softmax_probs(i, kval):
            sc_ = _dot_nt(q_s[i], kval) * scale
            m = jnp.max(sc_, axis=-1, keepdims=True)
            p = jnp.exp(sc_ - m)
            l = jnp.sum(p, axis=-1, keepdims=True)
            return p.astype(_BF16), l

        def issue_for(i, u):
            c = i // HPC
            part = (i % HPC) * NPART + u

            @pl.when(jnp.logical_and(i < NMAIN - HPC, part < NP))
            def _():
                issue_chunk_part(c + 1, part)

            e = i - (NMAIN - HPC)
            if u == 0:
                ep = jnp.where(e == 0, 0, e + 1)

                @pl.when(jnp.logical_and(e >= 0, ep < 2 * (LH - 1)))
                def _():
                    issue_last_part(ep // 2, ep % 2)

                @pl.when(e == 2 * (LH - 1))
                def _():
                    issue_last_head()
            else:
                @pl.when(e == 0)
                def _():
                    issue_last_part(0, 1)

        def step(i, carry):
            main = i < NMAIN
            hh = jnp.where(main, i % HPC, i - NMAIN)
            slot = jnp.where(main, (i // HPC) % NSLOT, LSLOT)
            blk = pl.ds(2 * hh, 2)

            issue_for(i, 0)

            @pl.when(jnp.logical_and(main, hh == 0))
            def _():
                _wait_full(kbuf.at[slot], ksem.at[slot])

            @pl.when(i >= NMAIN)
            def _():
                _wait_full(kbuf.at[LSLOT, blk], hsem.at[0, hh])

            p, l = softmax_probs(i, kbuf[slot, blk].reshape(Sk, Dh))

            issue_for(i, 1)

            @pl.when(jnp.logical_and(main, hh == 0))
            def _():
                _wait_full(vbuf.at[slot], vsem.at[slot])

            @pl.when(i >= NMAIN)
            def _():
                _wait_full(vbuf.at[LSLOT, blk], hsem.at[1, hh])

            o = _dot(p, vbuf[slot, blk].reshape(Sk, Dh)) / l
            h = i % H
            y = _dot(o.astype(_BF16), wo_v[h // 8, pl.ds(pl.multiple_of((h % 8) * Dh, Dh), Dh), :])
            acc_s[i // H] = acc_s[i // H] + y
            return carry

        jax.lax.fori_loop(0, BH - 1, step, 0)

        i = BH - 1
        b0 = 2 * (LH - 1)
        _wait_full(kbuf.at[LSLOT, pl.ds(b0, 2)], hsem.at[0, LH - 1])
        p, l = softmax_probs(i, kbuf[LSLOT, b0:b0 + 2].reshape(Sk, Dh))
        o = jnp.zeros((8, Dh), _F32)
        for pc in range(VPIECES):
            r0 = pc * PR
            _wait_full(vbuf.at[LSLOT, pl.ds(b0, 2), pl.ds(r0, PR)], lsem.at[pc])
            pp = jnp.concatenate([p[:, r0:r0 + PR], p[:, HS + r0:HS + r0 + PR]], axis=1)
            o = o + _dot(pp, vbuf[LSLOT, b0:b0 + 2, r0:r0 + PR, :].reshape(2 * PR, Dh))
        o = o / l
        y = _dot(o.astype(_BF16), wo_v[3, 7 * Dh:8 * Dh, :])
        a = jnp.concatenate([acc_s[0][0:1], acc_s[1][0:1] + y[0:1]], axis=0)
        out_v[...] = (gate * a + base).astype(out_v.dtype)
        c_out = pltpu.make_async_copy(out_v, out_hbm, osem.at[0])
        c_out.start()
        c_out.wait()

    any_spec = pl.BlockSpec(memory_space=pl.ANY)
    bf = _BF16
    out = pl.pallas_call(
        kernel,
        in_specs=[any_spec] * 11,
        out_specs=any_spec,
        out_shape=jax.ShapeDtypeStruct((B, D), A_x.dtype),
        scratch_shapes=[
            pltpu.VMEM((B, D), bf),
            pltpu.VMEM((D,), bf),
            pltpu.VMEM((4, D // 4, H * Dh), bf),
            pltpu.VMEM((4, H * Dh // 4, D), bf),
            pltpu.VMEM((B, NU, UR, Dc), bf),
            pltpu.VMEM((NJ, CH, Dh), bf),
            pltpu.VMEM((NJ, CH, Dh), bf),
            pltpu.VMEM((NJ, CH, Dh), bf),
            pltpu.VMEM((4, H * Dh // 4, M), bf),
            pltpu.VMEM((NSLOT, NBLK, HS, Dh), bf),
            pltpu.VMEM((NSLOT, NBLK, HS, Dh), bf),
            pltpu.VMEM((BH, 8, Dh), bf),
            pltpu.VMEM((B, 8, D), _F32),
            pltpu.VMEM((B, D), bf),
            pltpu.SemaphoreType.DMA((8,)),
            pltpu.SemaphoreType.DMA((B, NU)),
            pltpu.SemaphoreType.DMA((NSLOT,)),
            pltpu.SemaphoreType.DMA((NSLOT,)),
            pltpu.SemaphoreType.DMA((2, LH)),
            pltpu.SemaphoreType.DMA((VPIECES,)),
            pltpu.SemaphoreType.DMA((1,)),
        ],
        compiler_params=pltpu.CompilerParams(vmem_limit_bytes=110 * 1024 * 1024,
                                             disable_semaphore_checks=True),
    )(xa2, gate_w, k3, v3, wq2, wo2, ckv4, wqb2, wuk2, wuv2, wob2)
    return out.reshape(B, Sq, D)
```

```python
import jax
import jax.numpy as jnp
import jax.experimental.pallas as pl
import jax.experimental.pallas.tpu as pltpu

_NT = (((1,), (1,)), ((), ()))
_F32 = jnp.float32
_BF16 = jnp.bfloat16

NSLOT = 2
HPC = 5
LH = 4
NBLK = 2 * HPC
KVSUB = 16
LSUB = 48
NPART = 2
NP = 8
VPIECES = 4


def _dot(a, b):
    return jnp.dot(a, b, preferred_element_type=_F32)


def _dot_nt(a, b):
    return jax.lax.dot_general(a, b, _NT, preferred_element_type=_F32)


def _wait_full(buf, sem):
    pltpu.make_async_copy(buf, buf, sem).wait()


@jax.jit
def pallas_gated_mix__mha_block_cached__compressed_kv_cla__decode_kernel(
    A_x: jax.Array,
    A_k_cache: jax.Array,
    A_v_cache: jax.Array,
    A_wq: jax.Array,
    A_wo: jax.Array,
    B_x: jax.Array,
    B_c_kv: jax.Array,
    B_w_q: jax.Array,
    B_w_uk: jax.Array,
    B_w_uv: jax.Array,
    B_w_o: jax.Array,
    gate_w: jax.Array,
):
    B, Sq, D = A_x.shape
    _, H, Sk, Dh = A_k_cache.shape
    Dc = B_c_kv.shape[-1]
    M = B_w_q.shape[0]
    assert Sq == 1 and B == 2 and Dh == 128 and H == 32 and D == 512 and M == D and Dc == 512
    BH = B * H
    R = BH
    NJ = Dc // 128
    CH = 128 * H
    scale = float(Dh) ** -0.5
    NU = 8
    UR = Sk // NU
    UB = UR // NU
    QS = Sk // 4
    PR = QS // VPIECES

    xa2 = A_x.reshape(B, D)
    HS = Sk // 2
    NMAIN = BH - LH
    NCH = NMAIN // HPC
    assert NCH * HPC == NMAIN and NP <= NPART * HPC
    k3 = A_k_cache.reshape(2 * BH, 2, QS, Dh)
    v3 = A_v_cache.reshape(2 * BH, 2, QS, Dh)
    wqb2 = B_w_q.reshape(NJ, CH, Dh)
    wuk2 = B_w_uk.reshape(NJ, CH, Dh)
    wuv2 = B_w_uv.reshape(NJ, CH, Dh)
    wob2 = B_w_o.reshape(4, H * Dh // 4, M)
    wo2 = A_wo.reshape(4, H * Dh // 4, D)
    wq2 = A_wq.reshape(4, D // 4, H * Dh)
    ckv4 = B_c_kv.reshape(B, NU, UR, Dc)

    def kernel(xa_hbm, gw_hbm, k_hbm, v_hbm, wq_hbm, wo_hbm, ckv_hbm,
               wqb_hbm, wuk_hbm, wuv_hbm, wob_hbm,
               out_hbm,
               xa_v, gw_v, wq_v, wo_v, ckv_v, wqb_v, wuk_v, wuv_v, wob_v,
               kbuf, vbuf, q_s, acc_s, out_v,
               sem, csem, ksem, vsem, hsem, lsem, osem):

        def d_w3(src, dst, sm, t):
            r = pl.ds(pl.multiple_of(t * 32, 32), 32)
            return pltpu.make_async_copy(src.at[:, r], dst.at[:, r], sm)

        def d_w512(src, dst, sm, t):
            r = pl.ds(pl.multiple_of(t * 8, 8), 8)
            return pltpu.make_async_copy(src.at[:, r], dst.at[:, r], sm)

        def d_wq(src, dst, sm, t):
            r = pl.ds(pl.multiple_of((t // 8) * 8, 8), 8)
            c = pl.ds(pl.multiple_of((t % 8) * 512, 512), 512)
            return pltpu.make_async_copy(src.at[:, r, c], dst.at[:, r, c], sm)

        def d_ckv(src, dst, sm, t):
            r = pl.ds(pl.multiple_of((t // 2) * 8, 8), 8)
            c = pl.ds(pl.multiple_of((t % 2) * 256, 256), 256)
            return pltpu.make_async_copy(src.at[:, r, c], dst.at[:, r, c], sm)

        def issue_unit(d0, a0, d1, a1, u, n=32):
            def one(t, c):
                d1(*a1, t).start(priority=1)
                d0(*a0, t).start(priority=0)
                return c

            jax.lax.fori_loop(u * n, (u + 1) * n, one, 0, unroll=4)

        def issue_s1(u):
            issue_unit(d_w3, (wqb_hbm, wqb_v, sem.at[5]), d_w3, (wuk_hbm, wuk_v, sem.at[6]), u)

        def issue_ckv(u):
            issue_unit(d_ckv, (ckv_hbm.at[0], ckv_v.at[0], csem.at[0, u]),
                       d_ckv, (ckv_hbm.at[1], ckv_v.at[1], csem.at[1, u]), u, n=UB // 4)

        def issue_s3(u):
            issue_unit(d_w3, (wuv_hbm, wuv_v, sem.at[7]), d_w512, (wob_hbm, wob_v, sem.at[3]), u)

        def issue_s4(u):
            issue_unit(d_wq, (wq_hbm, wq_v, sem.at[2]), d_w512, (wo_hbm, wo_v, sem.at[4]), u)

        def kv_pairs(ksrc, kdst, ks, vsrc, vdst, vs, r0, rows, sub):
            nfull = rows // sub
            rem = rows - nfull * sub
            lead = (slice(None),) * (len(ksrc.shape) - 2)

            def pair(off, n):
                ix = lead + (pl.ds(off, n),)
                pltpu.make_async_copy(vsrc.at[ix], vdst.at[ix], vs).start(priority=1)
                pltpu.make_async_copy(ksrc.at[ix], kdst.at[ix], ks).start(priority=0)

            def one(t, c):
                pair(pl.multiple_of(r0 + t * sub, 16), sub)
                return c

            jax.lax.fori_loop(0, nfull, one, 0, unroll=4)
            if rem:
                pair(r0 + nfull * sub, rem)

        PROWS = HS // NP

        def issue_chunk_part(c, part):
            slot = c % NSLOT
            blk = pl.ds(c * NBLK, NBLK)
            q = part // (NP // 2)
            r0 = (part % (NP // 2)) * PROWS
            kv_pairs(k_hbm.at[blk, q], kbuf.at[slot, :, q], ksem.at[slot],
                     v_hbm.at[blk, q], vbuf.at[slot, :, q], vsem.at[slot], r0, PROWS, KVSUB)

        LSLOT = NCH % NSLOT

        def issue_last_part(hh, u):
            src = pl.ds(2 * (NMAIN + hh), 2)
            dst = pl.ds(2 * hh, 2)
            kv_pairs(k_hbm.at[src], kbuf.at[LSLOT, dst], hsem.at[0, hh],
                     v_hbm.at[src], vbuf.at[LSLOT, dst], hsem.at[1, hh],
                     u * (QS // NPART), QS // NPART, LSUB)

        def issue_last_head():
            hh = LH - 1
            src = pl.ds(2 * (NMAIN + hh), 2)
            dst = pl.ds(2 * hh, 2)
            for p in range(VPIECES):
                kv_pairs(k_hbm.at[src], kbuf.at[LSLOT, dst], hsem.at[0, hh],
                         v_hbm.at[src], vbuf.at[LSLOT, dst], lsem.at[p], p * PR, PR, LSUB)

        c_xa = pltpu.make_async_copy(xa_hbm, xa_v, sem.at[0])
        c_gw = pltpu.make_async_copy(gw_hbm, gw_v, sem.at[1])
        issue_s1(0)
        c_xa.start()
        c_gw.start()
        issue_s1(1)

        st = (jax.lax.broadcasted_iota(jnp.int32, (128, CH), 1) // H
              == jax.lax.broadcasted_iota(jnp.int32, (128, CH), 0)).astype(_F32).astype(_BF16)
        issue_s1(2)
        s_ = (jax.lax.broadcasted_iota(jnp.int32, (CH, 128), 0) // H
              == jax.lax.broadcasted_iota(jnp.int32, (CH, 128), 1)).astype(_F32).astype(_BF16)
        hmask = (jax.lax.broadcasted_iota(jnp.int32, (R, CH), 1) % H
                 == jax.lax.broadcasted_iota(jnp.int32, (R, CH), 0) % H)

        def project_j(c, w_ref, j):
            e = _dot(c[:, j * 128:(j + 1) * 128], st)
            l = jnp.where(hmask, e, 0.0).astype(_BF16)
            return _dot(l, w_ref[j])

        issue_s1(3)
        issue_ckv(0)
        issue_ckv(1)
        c_xa.wait()
        c_gw.wait()
        xav = xa_v[...].astype(_F32)
        xb = jnp.concatenate(
            [jnp.broadcast_to(xav[b:b + 1], (H, M)) for b in range(B)], axis=0).astype(_BF16)
        _wait_full(wqb_v, sem.at[5])
        qb = project_j(xb, wqb_v, 0) + project_j(xb, wqb_v, 1)
        issue_ckv(2)
        qb = qb + project_j(xb, wqb_v, 2) + project_j(xb, wqb_v, 3)
        qb = qb.astype(_BF16)

        def absorb_j(j):
            t = _dot_nt(qb, wuk_v[j])
            t = jnp.where(hmask, t, 0.0).astype(_BF16)
            return _dot(t, s_).astype(_BF16)

        issue_ckv(3)
        _wait_full(wuk_v, sem.at[6])
        qabs = [absorb_j(0), absorb_j(1)]
        issue_ckv(4)
        qabs += [absorb_j(2), absorb_j(3)]
        qabs = jnp.concatenate(qabs, axis=1)

        sc = [[None] * NU for _ in range(B)]

        def ckv_unit(b, u):
            return ckv_v[b, :, u * UB:(u + 1) * UB, :].reshape(NU * UB, Dc)

        def b_scores(u):
            for b in range(B):
                _wait_full(ckv_v.at[b, :, pl.ds(u * UB, UB)], csem.at[b, u])
                sc[b][u] = _dot_nt(qabs[b * H:(b + 1) * H], ckv_unit(b, u)) * scale

        def b_softmax(b):
            s = jnp.concatenate(sc[b], axis=1)
            m = jnp.max(s, axis=-1, keepdims=True)
            p = jnp.exp(s - m)
            l = jnp.sum(p, axis=-1, keepdims=True)
            return p.astype(_BF16), l

        def b_ctx(b, p, l):
            cc = _dot(p[:, 0:NU * UB], ckv_unit(b, 0))
            for u in range(1, NU):
                cc = cc + _dot(p[:, u * NU * UB:(u + 1) * NU * UB], ckv_unit(b, u))
            return (cc / l).astype(_BF16)

        issue_ckv(5)
        b_scores(0)
        b_scores(1)
        issue_ckv(6)
        b_scores(2)
        b_scores(3)
        issue_ckv(7)
        b_scores(4)
        b_scores(5)
        issue_s3(0)
        b_scores(6)
        issue_s3(1)
        b_scores(7)
        p0, l0 = b_softmax(0)
        issue_s3(2)
        p1, l1 = b_softmax(1)
        issue_s3(3)
        cc0 = b_ctx(0, p0, l0)
        issue_s4(0)
        cc1 = b_ctx(1, p1, l1)
        ctxc = jnp.concatenate([cc0, cc1], axis=0)
        issue_s4(1)
        _wait_full(wuv_v, sem.at[7])
        ctx = project_j(ctxc, wuv_v, 0) + project_j(ctxc, wuv_v, 1)
        issue_s4(2)
        ctx = ctx + project_j(ctxc, wuv_v, 2) + project_j(ctxc, wuv_v, 3)
        issue_s4(3)

        _wait_full(wob_v, sem.at[3])
        dmask = (jax.lax.broadcasted_iota(jnp.int32, (R, H * Dh), 1) // Dh
                 == jax.lax.broadcasted_iota(jnp.int32, (R, H * Dh), 0) % H)
        l2 = jnp.where(dmask, jnp.tile(ctx, (1, H)), 0.0).astype(_BF16)
        yb = _dot(l2, wob_v[...].reshape(H * Dh, M))
        outb = [jnp.sum(yb[b * H:(b + 1) * H], axis=0, keepdims=True) for b in range(B)]
        issue_chunk_part(0, 0)

        gw = gw_v[...].astype(_F32).reshape(1, D)
        gate = jax.nn.sigmoid(jnp.sum(xav * gw, axis=-1, keepdims=True))
        base = (1.0 - gate) * jnp.concatenate(outb, axis=0)
        issue_chunk_part(0, 1)

        _wait_full(wq_v, sem.at[2])
        xa = jnp.concatenate(
            [jnp.broadcast_to(xav[b:b + 1], (8, D)) for b in range(B)], axis=0).astype(_BF16)
        qa = _dot(xa, wq_v[...].reshape(D, H * Dh))
        for b in range(B):
            for h in range(H):
                q_s[b * H + h] = qa[b * 8:(b + 1) * 8, h * Dh:(h + 1) * Dh].astype(_BF16)
        acc_s[...] = jnp.zeros_like(acc_s)
        for part in range(2, NP):
            issue_chunk_part(0, part)
        _wait_full(wo_v, sem.at[4])

        def softmax_probs(i, kval):
            sc_ = _dot_nt(q_s[i], kval) * scale
            m = jnp.max(sc_, axis=-1, keepdims=True)
            p = jnp.exp(sc_ - m)
            l = jnp.sum(p, axis=-1, keepdims=True)
            return p.astype(_BF16), l

        def issue_for(i, u):
            c = i // HPC
            part = (i % HPC) * NPART + u

            @pl.when(jnp.logical_and(i < NMAIN - HPC, part < NP))
            def _():
                issue_chunk_part(c + 1, part)

            e = i - (NMAIN - HPC)
            if u == 0:
                ep = jnp.where(e == 0, 0, e + 1)

                @pl.when(jnp.logical_and(e >= 0, ep < 2 * (LH - 1)))
                def _():
                    issue_last_part(ep // 2, ep % 2)

                @pl.when(e == 2 * (LH - 1))
                def _():
                    issue_last_head()
            else:
                @pl.when(e == 0)
                def _():
                    issue_last_part(0, 1)

        def step(i, carry):
            main = i < NMAIN
            hh = jnp.where(main, i % HPC, i - NMAIN)
            slot = jnp.where(main, (i // HPC) % NSLOT, LSLOT)
            blk = pl.ds(2 * hh, 2)

            issue_for(i, 0)

            @pl.when(jnp.logical_and(main, hh == 0))
            def _():
                _wait_full(kbuf.at[slot], ksem.at[slot])

            @pl.when(i >= NMAIN)
            def _():
                _wait_full(kbuf.at[LSLOT, blk], hsem.at[0, hh])

            p, l = softmax_probs(i, kbuf[slot, blk].reshape(Sk, Dh))

            issue_for(i, 1)

            @pl.when(jnp.logical_and(main, hh == 0))
            def _():
                _wait_full(vbuf.at[slot], vsem.at[slot])

            @pl.when(i >= NMAIN)
            def _():
                _wait_full(vbuf.at[LSLOT, blk], hsem.at[1, hh])

            o = _dot(p, vbuf[slot, blk].reshape(Sk, Dh)) / l
            h = i % H
            y = _dot(o.astype(_BF16), wo_v[h // 8, pl.ds(pl.multiple_of((h % 8) * Dh, Dh), Dh), :])
            acc_s[i // H] = acc_s[i // H] + y
            return carry

        jax.lax.fori_loop(0, BH - 1, step, 0)

        i = BH - 1
        b0 = 2 * (LH - 1)
        _wait_full(kbuf.at[LSLOT, pl.ds(b0, 2)], hsem.at[0, LH - 1])
        p, l = softmax_probs(i, kbuf[LSLOT, b0:b0 + 2].reshape(Sk, Dh))
        o = jnp.zeros((8, Dh), _F32)
        for pc in range(VPIECES):
            r0 = pc * PR
            _wait_full(vbuf.at[LSLOT, pl.ds(b0, 2), :, pl.ds(r0, PR)], lsem.at[pc])
            pp = jnp.concatenate([p[:, q * QS + r0:q * QS + r0 + PR] for q in range(4)], axis=1)
            o = o + _dot(pp, vbuf[LSLOT, b0:b0 + 2, :, r0:r0 + PR, :].reshape(4 * PR, Dh))
        o = o / l
        y = _dot(o.astype(_BF16), wo_v[3, 7 * Dh:8 * Dh, :])
        a = jnp.concatenate([acc_s[0][0:1], acc_s[1][0:1] + y[0:1]], axis=0)
        out_v[...] = (gate * a + base).astype(out_v.dtype)
        c_out = pltpu.make_async_copy(out_v, out_hbm, osem.at[0])
        c_out.start()
        c_out.wait()

    any_spec = pl.BlockSpec(memory_space=pl.ANY)
    bf = _BF16
    out = pl.pallas_call(
        kernel,
        in_specs=[any_spec] * 11,
        out_specs=any_spec,
        out_shape=jax.ShapeDtypeStruct((B, D), A_x.dtype),
        scratch_shapes=[
            pltpu.VMEM((B, D), bf),
            pltpu.VMEM((D,), bf),
            pltpu.VMEM((4, D // 4, H * Dh), bf),
            pltpu.VMEM((4, H * Dh // 4, D), bf),
            pltpu.VMEM((B, NU, UR, Dc), bf),
            pltpu.VMEM((NJ, CH, Dh), bf),
            pltpu.VMEM((NJ, CH, Dh), bf),
            pltpu.VMEM((NJ, CH, Dh), bf),
            pltpu.VMEM((4, H * Dh // 4, M), bf),
            pltpu.VMEM((NSLOT, NBLK, 2, QS, Dh), bf),
            pltpu.VMEM((NSLOT, NBLK, 2, QS, Dh), bf),
            pltpu.VMEM((BH, 8, Dh), bf),
            pltpu.VMEM((B, 8, D), _F32),
            pltpu.VMEM((B, D), bf),
            pltpu.SemaphoreType.DMA((8,)),
            pltpu.SemaphoreType.DMA((B, NU)),
            pltpu.SemaphoreType.DMA((NSLOT,)),
            pltpu.SemaphoreType.DMA((NSLOT,)),
            pltpu.SemaphoreType.DMA((2, LH)),
            pltpu.SemaphoreType.DMA((VPIECES,)),
            pltpu.SemaphoreType.DMA((1,)),
        ],
        compiler_params=pltpu.CompilerParams(vmem_limit_bytes=110 * 1024 * 1024,
                                             disable_semaphore_checks=True),
    )(xa2, gate_w, k3, v3, wq2, wo2, ckv4, wqb2, wuk2, wuv2, wob2)
    return out.reshape(B, Sq, D)
```
